```python
import jax
import jax.numpy as jnp

def _softmax(x, axis=-1):
    return jax.nn.softmax(x, axis=axis)
def _gelu(x):
    return jax.nn.gelu(x, approximate=True)
def _silu(x):
    return jax.nn.silu(x)
def _sigmoid(x):
    return jax.nn.sigmoid(x)
def _layernorm(x, axis=-1, eps=1e-5):
    m = jnp.mean(x, axis=axis, keepdims=True)
    v = jnp.var(x, axis=axis, keepdims=True)
    return (x - m) / jnp.sqrt(v + eps)
def _scatter_add(tgt, idx, src, axis=0):
    return tgt.at[idx].add(src)
def _segment_sum(src, seg, n):
    return jax.ops.segment_sum(src, seg, n)
class _Rng:
    def __init__(self, key):
        self._k = key
    def _next(self):
        self._k, sub = jax.random.split(self._k)
        return sub
    def normal(self, shape):
        return jax.random.normal(self._next(), shape, dtype=jnp.bfloat16)
    def randint(self, lo, hi, shape):
        return jax.random.randint(self._next(), shape, lo, hi, dtype=jnp.int32)
    def uniform(self, shape, lo=0.0, hi=1.0):
        return jax.random.uniform(self._next(), shape, jnp.bfloat16, lo, hi)
    def permutation(self, n):
        return jax.random.permutation(self._next(), n)


kernel_name = 'interleave_layers__linear_kernel_hedgehog__sliding_local_dilated__prompt'

def setup_inputs():
    _rng = _Rng(jax.random.key(int.from_bytes(__import__("os").urandom(4), "little")))
    _w = (lambda a: (lambda t: t.astype(jnp.bfloat16) if jnp.issubdtype(t.dtype, jnp.floating) else t)(jnp.asarray(a)))
    def _A_setup():
        B, S, D, H = 1, 2048, 1024, 32
        Dh = D // H
        return {
            "x": _w((lambda *s: _rng.normal(s) * 0.05)(B, S, D)),
            "wqkv": _w((lambda *s: _rng.normal(s) * 0.05)(D, 3 * D)),
            "w_phi": _w((lambda *s: _rng.normal(s) * 0.05)(H, Dh, Dh) * (Dh ** -0.5)),
            "wo": _w((lambda *s: _rng.normal(s) * 0.05)(D, D)),
        }
    _A_in = _A_setup()

    def _B_setup():
        B, S, D = 1, 2048, 1024
        return {
            "x": _w((lambda *s: _rng.normal(s) * 0.05)(B, S, D)),
            "wqkv": _w((lambda *s: _rng.normal(s) * 0.05)(D, 3 * D)),
            "wo": _w((lambda *s: _rng.normal(s) * 0.05)(D, D)),
        }
    _B_in = _B_setup()

    return {
        "A_x": _A_in["x"],
        "A_wqkv": _A_in["wqkv"],
        "A_w_phi": _A_in["w_phi"],
        "A_wo": _A_in["wo"],
        "B_x": _B_in["x"],
        "B_wqkv": _B_in["wqkv"],
        "B_wo": _B_in["wo"],
    }

def reference(A_x, A_wqkv, A_w_phi, A_wo, B_x, B_wqkv, B_wo):
    def _A_ref(x, wqkv, w_phi, wo):
        B, S, D = x.shape
        H = 32; Dh = D // H
        qkv = (lambda x, *d: x.transpose(*d))((x @ wqkv).reshape(B, S, 3, H, Dh), 2, 0, 3, 1, 4)
        q, k, v = qkv[0], qkv[1], qkv[2]
        pq = jnp.einsum("bhsd,hdf->bhsf", q, w_phi)
        pk = jnp.einsum("bhsd,hdf->bhsf", k, w_phi)
        phi_q = jnp.concatenate([_softmax(pq, axis=-1), _softmax(-pq, axis=-1)], axis=-1)
        phi_k = jnp.concatenate([_softmax(pk, axis=-1), _softmax(-pk, axis=-1)], axis=-1)
        kv = jnp.einsum("bhsf,bhsd->bhfd", phi_k, v)
        z  = jnp.einsum("bhsf->bhf", phi_k)
        num = jnp.einsum("bhqf,bhfd->bhqd", phi_q, kv)
        den = jnp.einsum("bhqf,bhf->bhq", phi_q, z)[..., None] + 1e-6
        o = num / den
        return (lambda x, *d: x.transpose(*d))(o, 0, 2, 1, 3).reshape(B, S, D) @ wo

    def _B_ref(x, wqkv, wo):
        B, S, D = x.shape
        H = 32; Dh = D // H
        W, dil = 8, 2
        qkv = (lambda x, *d: x.transpose(*d))((x @ wqkv).reshape(B, S, 3, H, Dh), 2, 0, 3, 1, 4)
        q, k, v = qkv[0], qkv[1], qkv[2]
        scale = Dh ** -0.5
        pos = jnp.arange(S)
        off = jnp.arange(W) * dil
        idx = pos[:, None] - off[None, :]
        mask = idx >= 0
        idx_c = jnp.where(mask, idx, 0).reshape(-1)
        kg = k[:, :, idx_c, :].reshape(B, H, S, W, Dh)
        vg = v[:, :, idx_c, :].reshape(B, H, S, W, Dh)
        logits = jnp.einsum("bhsd,bhswd->bhsw", q, kg) * scale
        logits = jnp.where(mask[None, None, :, :], logits, -1e9)
        attn = _softmax(logits, axis=-1)
        o = jnp.einsum("bhsw,bhswd->bhsd", attn, vg)
        return (lambda x, *d: x.transpose(*d))(o, 0, 2, 1, 3).reshape(B, S, D) @ wo

    x = A_x
    x = x + _A_ref(_layernorm(x, axis=-1), A_wqkv, A_w_phi, A_wo)
    x = x + _B_ref(_layernorm(x, axis=-1), B_wqkv, B_wo)
    x = x + _A_ref(_layernorm(x, axis=-1), A_wqkv, A_w_phi, A_wo)
    x = x + _B_ref(_layernorm(x, axis=-1), B_wqkv, B_wo)
    return x
```

```python
import functools

import jax
import jax.numpy as jnp
from jax import lax
import jax.experimental.pallas as pl
import jax.experimental.pallas.tpu as pltpu

F32, BF16, U32 = jnp.float32, jnp.bfloat16, jnp.uint32
S, D, H, DH = 2048, 1024, 32, 32
NT = S // 128
NC = 256
NCH = S // NC
LOG2E = 1.4426950408889634
NT_DIMS = (((1,), (1,)), ((), ()))


def _dot(a, b):
    return jnp.dot(a, b, preferred_element_type=F32)


def _dot_nt(a, b):
    return lax.dot_general(a, b, NT_DIMS, preferred_element_type=F32)


def _interleave(main, n_main, *sides):
    done = [0] * len(sides)
    for i in range(n_main):
        next(main)
        for k, (g, n) in enumerate(sides):
            while done[k] < (i + 1) * n // n_main:
                next(g)
                done[k] += 1
    for g in (main,) + tuple(g for g, _ in sides):
        for _ in g:
            raise AssertionError("generator piece count mismatch")


def _drain(g):
    for _ in g:
        pass


def _red_h2(x, op):
    r = op(x[0], x[1])
    for i in range(2, 8):
        r = op(r, x[i])
    r = op(r, pltpu.roll(r, 4, 0))
    r = op(r, pltpu.roll(r, 2, 0))
    return r[None]


def _hedgehog(p):
    n = p.shape[1]
    p3 = p.reshape(8, 8, n)
    mx = _red_h2(p3, jnp.maximum)
    mn = _red_h2(p3, jnp.minimum)
    e1 = jnp.exp2(p3 - mx)
    e2 = jnp.exp2(mn - p3)
    s1 = _red_h2(e1, jnp.add)
    s2 = _red_h2(e2, jnp.add)
    a = (e1 * pl.reciprocal(s1, approx=True)).reshape(64, n)
    b = (e2 * pl.reciprocal(s2, approx=True)).reshape(64, n)
    return a, b


def _ln_pieces(xT, xnT, c0, n):
    rows = [slice(m * 128, (m + 1) * 128) for m in range(8)]
    cols = pl.ds(c0, n)
    s = None
    for r in rows:
        t = jnp.sum(xT[r, cols].reshape(16, 8, n), axis=0)
        s = t if s is None else s + t
        yield
    mean = jnp.sum(s, axis=0, keepdims=True) * (1.0 / D)
    s = None
    for r in rows:
        d = xT[r, cols] - mean
        t = jnp.sum((d * d).reshape(16, 8, n), axis=0)
        s = t if s is None else s + t
        yield
    rstd = lax.rsqrt(jnp.sum(s, axis=0, keepdims=True) * (1.0 / D) + 1e-5)
    for r in rows:
        xnT[r, cols] = ((xT[r, cols] - mean) * rstd).astype(BF16)
        yield


N_LN = 24


def _kernel(x_hbm, wa_hbm, wphi_ref, woa_hbm, wb_hbm, wob_hbm, out_ref,
            xs, wraw, wraw_o, tmp,
            xT, xnT, oT, wa_kv, wa_q, woT, wb,
            kvacc, zacc, kvm, qbuf, kbuf, vbuf, sems):

    x_cp = [pltpu.make_async_copy(x_hbm.at[:, i * 128:(i + 1) * 128], xs.at[i], sems.at[i])
            for i in range(8)]
    wa_cp = pltpu.make_async_copy(wa_hbm, wraw.at[0], sems.at[8])
    wb_cp = pltpu.make_async_copy(wb_hbm, wraw.at[1], sems.at[9])
    woa_cp = pltpu.make_async_copy(woa_hbm, wraw_o.at[0], sems.at[10])
    wob_cp = pltpu.make_async_copy(wob_hbm, wraw_o.at[1], sems.at[11])
    for c in x_cp:
        c.start()
    wa_cp.start()
    woa_cp.start()
    wb_cp.start()
    wob_cp.start()

    qbuf[...] = jnp.zeros(qbuf.shape, F32)
    kbuf[...] = jnp.zeros(kbuf.shape, F32)
    vbuf[...] = jnp.zeros(vbuf.shape, F32)

    for c in x_cp:
        c.wait()
    xu = xs.bitcast(U32)
    for r in range(8):
        for i in range(8):
            t = xu[i, pl.ds(r, 128, stride=8), :].T
            rows = slice(i * 128, (i + 1) * 128)
            xT[rows, r * 128:(r + 1) * 128] = pltpu.bitcast(t << 16, F32)
            xT[rows, 1024 + r * 128:1024 + (r + 1) * 128] = pltpu.bitcast(
                t & jnp.uint32(0xFFFF0000), F32)

    def ln_only(j, _):
        _drain(_ln_pieces(xT, xnT, pl.multiple_of(j * NC, NC), NC))
        return _
    lax.fori_loop(0, NCH, ln_only, None)

    row = lax.broadcasted_iota(jnp.int32, (128, 128), 0)
    col = lax.broadcasted_iota(jnp.int32, (128, 128), 1)
    src_head = 2 * (row // 64) + row % 2
    src_j = (row % 64) // 2
    perm_h2 = ((src_head * 32 + src_j) == col).astype(BF16)
    sel_f = (lax.broadcasted_iota(jnp.int32, (128, 32), 0) % 64 // 2
             == lax.broadcasted_iota(jnp.int32, (128, 32), 1)).astype(BF16)

    wa_cp.wait()

    def prep_a(blk, _):
        c0 = pl.multiple_of(blk * 128, 128)
        wphi = wphi_ref[pl.ds(c0, 128), :]
        fold = jnp.where(src_head == col // 32, _dot_nt(sel_f, wphi), 0.0).astype(BF16)
        q = _dot_nt(fold, wraw[0, :, pl.ds(c0, 128)]) * LOG2E
        wa_q[pl.ds(c0, 128), :] = q.astype(BF16)
        k = (_dot_nt(fold, wraw[0, :, pl.ds(D + c0, 128)]) * LOG2E).astype(BF16)
        v = _dot_nt(perm_h2, wraw[0, :, pl.ds(2 * D + c0, 128)]).astype(BF16)
        r0 = pl.multiple_of(blk * 256, 256)
        wa_kv[pl.ds(r0, 64), :] = k[:64]
        wa_kv[pl.ds(r0 + 64, 64), :] = v[:64]
        wa_kv[pl.ds(r0 + 128, 64), :] = k[64:]
        wa_kv[pl.ds(r0 + 192, 64), :] = v[64:]
        return _
    lax.fori_loop(0, 8, prep_a, None)

    woa_cp.wait()

    def prep_woa(blk, _):
        c0 = pl.multiple_of(blk * 128, 128)
        wp = _dot(perm_h2, wraw_o[0, pl.ds(c0, 128), :])
        woT[0, :, pl.ds(c0, 128)] = wp.astype(BF16).T
        return _
    lax.fori_loop(0, 8, prep_woa, None)

    wob_cp.wait()
    wb_cp.wait()

    def prep_wob(hg, _):
        r0 = pl.multiple_of(hg * 256, 256)
        w = wraw_o[1, pl.ds(r0, 256), :].astype(F32)
        for i in range(8):
            tmp[i] = w[:, i * 128:(i + 1) * 128]
        for i in range(8):
            wp = jnp.concatenate([tmp[i, pl.ds(d, 8, stride=32), :] for d in range(32)], axis=0)
            woT[1, i * 128:(i + 1) * 128, pl.ds(r0, 256)] = wp.astype(BF16).T
        return _
    lax.fori_loop(0, 4, prep_wob, None)

    def prep_wb(i, _):
        part, hg = i // 4, i % 4
        c0 = pl.multiple_of(part * D + hg * 256, 256)
        t = wraw[1, :, pl.ds(c0, 256)].astype(F32).T
        for k in range(8):
            tmp[k] = t[:, k * 128:(k + 1) * 128]
        r0 = pl.multiple_of(hg * 768 + part * 256, 256)
        for k in range(8):
            wp = jnp.concatenate([tmp[k, pl.ds(d, 8, stride=32), :] for d in range(32)], axis=0)
            wb[pl.ds(r0, 256), k * 128:(k + 1) * 128] = wp.astype(BF16)
        return _
    lax.fori_loop(0, 12, prep_wb, None)

    def a_phase1(j, _):
        cols = pl.ds(pl.multiple_of(j * NC, NC), NC)
        pend = None
        for gg in range(17):
            res = None
            if gg < 16:
                res = _dot(wa_kv[gg * 128:(gg + 1) * 128, :], xnT[:, cols])
            if pend is not None:
                g = gg - 1
                a, b = _hedgehog(pend[:64])
                phi = jnp.concatenate([a, b], axis=0)
                zacc[g * 128:(g + 1) * 128, :] += phi[:, :128] + phi[:, 128:]
                kvacc[g * 64:(g + 1) * 64, :] += _dot_nt(pend[64:].astype(BF16), phi.astype(BF16))
            pend = res
        return _

    def a_finalize(g, _):
        r0 = pl.multiple_of(g * 128, 128)
        z = jnp.sum(zacc[pl.ds(r0, 128), :], axis=1, keepdims=True)
        zacc[pl.ds(r0, 128), :] = jnp.broadcast_to(z, (128, 128))
        r1 = pl.multiple_of(g * 64, 64)
        same = (lax.broadcasted_iota(jnp.int32, (64, 128), 0) % 2
                == lax.broadcasted_iota(jnp.int32, (64, 128), 1) % 2)
        kvm[pl.ds(r1, 64), :] = jnp.where(same, kvacc[pl.ds(r1, 64), :], 0.0).astype(BF16)
        return _

    def a_phase2(j, _):
        cols = pl.ds(pl.multiple_of(j * NC, NC), NC)
        pq, pn = None, None
        for gg in range(18):
            res = None
            if gg < 16:
                res = _dot(wa_q[gg * 64:(gg + 1) * 64, :], xnT[:, cols])
            num = None
            if pq is not None and gg - 1 < 16:
                g = gg - 1
                a, b = _hedgehog(pq)
                za = zacc[g * 128:g * 128 + 64, :]
                zb = zacc[g * 128 + 64:(g + 1) * 128, :]
                za = jnp.concatenate([za, za], axis=1)
                zb = jnp.concatenate([zb, zb], axis=1)
                den = _red_h2((a * za + b * zb).reshape(8, 8, NC), jnp.add)
                inv = pl.reciprocal(den + 1e-6, approx=True)
                phi = jnp.concatenate([a, b], axis=0).astype(BF16)
                num = (_dot(kvm[g * 64:(g + 1) * 64, :], phi), inv)
            if pn is not None:
                g = gg - 2
                n_, inv_ = pn
                o = (n_.reshape(8, 8, NC) * inv_).reshape(64, NC)
                oT[g * 64:(g + 1) * 64, cols] = o.astype(BF16)
            pq, pn = res, num
        return _

    def qkv_pieces(par, hg, slot):
        for n in range(4):
            cols = pl.ds(pl.multiple_of(par * 1024 + n * NC, NC), NC)
            for m in range(6):
                r0 = pl.multiple_of(hg * 768 + m * 128, 128)
                res = _dot(wb[pl.ds(r0, 128), :], xnT[:, cols])
                rr = slice((m % 2) * 128, (m % 2) * 128 + 128)
                if m < 2:
                    qbuf[slot, rr, n * NC:(n + 1) * NC] = res
                else:
                    buf = kbuf if m < 4 else vbuf
                    buf[slot, rr, 896 + n * NC:896 + (n + 1) * NC] = res
                    for t in range(2 * n, 2 * n + 2):
                        if t >= 1:
                            sh = pltpu.roll(res[:, (t % 2) * 128:(t % 2) * 128 + 128], 1, 1)
                            buf[slot, rr, (t - 1) * 128:t * 128] = sh
                yield

    N_QKV = 24
    lane0 = lax.broadcasted_iota(jnp.int32, (8, 128), 1) == 0

    def attn_pieces(par, hg, slot):
        scale = DH ** -0.5 * LOG2E
        for rp in range(0, 8, 2):
            logit = [[None] * 8, [None] * 8]
            for dd in range(0, 32, 8):
                for d in range(dd, dd + 8):
                    rows = slice(d * 8, d * 8 + 8)
                    q = [qbuf[slot, rows, (rp + a) * 128:(rp + a + 1) * 128] for a in range(2)]
                    for e in range(rp, rp + 9):
                        k = kbuf[slot, rows, e * 128:(e + 1) * 128]
                        for a in range(2):
                            w = rp + a + 7 - e
                            if 0 <= w < 8:
                                t = q[a] * k
                                logit[a][w] = t if logit[a][w] is None else logit[a][w] + t
                yield
            prob = []
            for a in range(2):
                lg = []
                for w in range(8):
                    t = logit[a][w] * scale
                    if w > rp + a:
                        t = jnp.where(lane0, -1e9 * LOG2E, t)
                    lg.append(t)
                mx = functools.reduce(jnp.maximum, lg)
                ex = [jnp.exp2(t - mx) for t in lg]
                inv = pl.reciprocal(functools.reduce(jnp.add, ex), approx=True)
                prob.append([t * inv for t in ex])
            yield
            for dd in range(0, 32, 2):
                outs = []
                for d in (dd, dd + 1):
                    rows = slice(d * 8, d * 8 + 8)
                    acc = [None, None]
                    for e in range(rp, rp + 9):
                        v = vbuf[slot, rows, e * 128:(e + 1) * 128]
                        for a in range(2):
                            w = rp + a + 7 - e
                            if 0 <= w < 8:
                                t = prob[a][w] * v
                                acc[a] = t if acc[a] is None else acc[a] + t
                    outs.append(jnp.concatenate(acc, axis=1))
                o = jnp.concatenate(outs, axis=0).astype(BF16)
                r0 = pl.multiple_of(hg * 256 + dd * 8, 16)
                c0 = pl.multiple_of(par * 1024 + rp * 128, 256)
                oT[pl.ds(r0, 16), pl.ds(c0, 256)] = o
                if dd % 8 == 6:
                    yield

    N_ATTN = 4 * 9

    def b_unit(i, _):
        prev = (i + 7) % 8
        _interleave(qkv_pieces(i // 4, i % 4, i % 2), N_QKV,
                    (attn_pieces(prev // 4, prev % 4, prev % 2), N_ATTN))
        return _

    def oproj_pieces(layer, cols):
        for m in range(8):
            rows = slice(m * 128, (m + 1) * 128)
            xT[rows, cols] += _dot(woT[layer % 2, rows, :], oT[:, cols])
            yield

    def o_chunk(layer, j, _):
        cols = pl.ds(pl.multiple_of(j * NC, NC), NC)
        prev = pl.multiple_of(((j + NCH - 1) % NCH) * NC, NC)
        _interleave(oproj_pieces(layer, cols), 8, (_ln_pieces(xT, xnT, prev, NC), N_LN))
        return _

    def layer_body(layer, _):
        @pl.when(layer % 2 == 0)
        def _a():
            kvacc[...] = jnp.zeros(kvacc.shape, F32)
            zacc[...] = jnp.zeros(zacc.shape, F32)
            lax.fori_loop(0, NCH, a_phase1, None)
            lax.fori_loop(0, 16, a_finalize, None)
            lax.fori_loop(0, NCH, a_phase2, None)

        @pl.when(layer % 2 == 1)
        def _b():
            lax.fori_loop(0, 8, b_unit, None)
            _drain(attn_pieces(1, 3, 1))

        lax.fori_loop(0, NCH, functools.partial(o_chunk, layer), None)
        _drain(_ln_pieces(xT, xnT, (NCH - 1) * NC, NC))
        return _

    lax.fori_loop(0, 4, layer_body, None)

    ou = xs.bitcast(U32)
    for r in range(8):
        for i in range(8):
            rows = slice(i * 128, (i + 1) * 128)
            w = pltpu.pack_elementwise(
                [xT[rows, r * 128:(r + 1) * 128], xT[rows, 1024 + r * 128:1024 + (r + 1) * 128]],
                packed_dtype=BF16)
            ou[i, pl.ds(r, 128, stride=8), :] = w.T
    o_cp = [pltpu.make_async_copy(xs.at[i], out_ref.at[:, i * 128:(i + 1) * 128], sems.at[i])
            for i in range(8)]
    for c in o_cp:
        c.start()
    for c in o_cp:
        c.wait()


@jax.jit
def pallas_interleave_layers__linear_kernel_hedgehog__sliding_local_dilated__prompt_kernel(
    A_x: jax.Array,
    A_wqkv: jax.Array,
    A_w_phi: jax.Array,
    A_wo: jax.Array,
    B_x: jax.Array,
    B_wqkv: jax.Array,
    B_wo: jax.Array,
):
    del B_x
    hbm = pl.BlockSpec(memory_space=pl.ANY)
    out = pl.pallas_call(
        _kernel,
        out_shape=jax.ShapeDtypeStruct((S, D), BF16),
        in_specs=[hbm, hbm, pl.BlockSpec(memory_space=pltpu.VMEM), hbm, hbm, hbm],
        out_specs=hbm,
        scratch_shapes=[
            pltpu.VMEM((8, S, 128), BF16),
            pltpu.VMEM((2, D, 3 * D), BF16),
            pltpu.VMEM((2, D, D), BF16),
            pltpu.VMEM((8, 256, 128), F32),
            pltpu.VMEM((D, S), F32),
            pltpu.VMEM((D, S), BF16),
            pltpu.VMEM((D, S), BF16),
            pltpu.VMEM((2 * D, D), BF16),
            pltpu.VMEM((D, D), BF16),
            pltpu.VMEM((2, D, D), BF16),
            pltpu.VMEM((3 * D, D), BF16),
            pltpu.VMEM((D, 128), F32),
            pltpu.VMEM((2 * D, 128), F32),
            pltpu.VMEM((D, 128), BF16),
            pltpu.VMEM((2, 256, 1024), F32),
            pltpu.VMEM((2, 256, 1920), F32),
            pltpu.VMEM((2, 256, 1920), F32),
            pltpu.SemaphoreType.DMA((12,)),
        ],
        compiler_params=pltpu.CompilerParams(vmem_limit_bytes=110 * 2**20),
    )(A_x.reshape(S, D), A_wqkv, A_w_phi.reshape(H * DH, DH), A_wo, B_wqkv, B_wo)
    return out.reshape(1, S, D)
```

```python
import functools

import jax
import jax.numpy as jnp
from jax import lax
import jax.experimental.pallas as pl
import jax.experimental.pallas.tpu as pltpu

F32, BF16, U32 = jnp.float32, jnp.bfloat16, jnp.uint32
S, D, H, DH = 2048, 1024, 32, 32
NT = S // 128
NC = 256
NCH = S // NC
LOG2E = 1.4426950408889634
KOFF, VOFF, QDUM = 1024, 1024 + 1920, 1024 + 2 * 1920
PAD = NC
DUM = PAD + S
CFG = {}
def cfg(k, d): return CFG.get(k, d)
OM = cfg("OM", 32)
OPIPE = cfg("OPIPE", 0)
QM = cfg("QM", 128)
QPIPE = cfg("QPIPE", 0)
NT_DIMS = (((1,), (1,)), ((), ()))


def _dot(a, b):
    return jnp.dot(a, b, preferred_element_type=F32)


def _dot_nt(a, b):
    return lax.dot_general(a, b, NT_DIMS, preferred_element_type=F32)


def _ld(ref, rows, cols=slice(None), lead=()):
    if isinstance(rows, slice):
        a = rows.start or 0
        rows = slice(a // 2, None if rows.stop is None else rows.stop // 2)
    else:
        start, size = rows
        rows = pl.ds(pl.multiple_of(start // 2, 8), size // 2)
    return pltpu.bitcast(ref[lead + (rows, cols)], BF16)


def _st(ref, rows, cols, val, lead=()):
    if isinstance(rows, slice):
        rows = slice(rows.start // 2, rows.stop // 2)
    else:
        start, size = rows
        rows = pl.ds(pl.multiple_of(start // 2, 8), size // 2)
    ref[lead + (rows, cols)] = pltpu.bitcast(val, U32)


def _interleave(main, n_main, *sides, lead=0):
    done = [0] * len(sides)
    for i in range(n_main):
        next(main)
        for k, (g, n) in enumerate(sides):
            while done[k] < min(n, (i + 1) * n // (n_main - lead)):
                next(g)
                done[k] += 1
    for g in (main,) + tuple(g for g, _ in sides):
        for _ in g:
            raise AssertionError("generator piece count mismatch")


def _drain(g):
    for _ in g:
        pass


def _red_h2(x, op):
    r = op(x[0], x[1])
    for i in range(2, 8):
        r = op(r, x[i])
    r = op(r, pltpu.roll(r, 4, 0))
    r = op(r, pltpu.roll(r, 2, 0))
    return r[None]


def _hedgehog(p):
    n = p.shape[1]
    p3 = p.reshape(8, 8, n)
    mx = _red_h2(p3, jnp.maximum)
    mn = _red_h2(p3, jnp.minimum)
    e1 = jnp.exp2(p3 - mx)
    e2 = jnp.exp2(mn - p3)
    s1 = _red_h2(e1, jnp.add)
    s2 = _red_h2(e2, jnp.add)
    a = (e1 * pl.reciprocal(s1, approx=True)).reshape(64, n)
    b = (e2 * pl.reciprocal(s2, approx=True)).reshape(64, n)
    return a, b


def _ln_pieces(xT, xnT, cols, lm, pin=None):
    n = cols.size if isinstance(cols, pl.Slice) else cols.stop - cols.start
    rows = [slice(m * lm, (m + 1) * lm) for m in range(D // lm)]
    s = None
    for r in rows:
        t = jnp.sum(xT[r, cols].reshape(lm // 8, 8, n), axis=0)
        s = t if s is None else s + t
        if pin is not None:
            xnT[0:8, pin] = pltpu.bitcast(s, U32)
        yield
    mean = jnp.sum(s, axis=0, keepdims=True) * (1.0 / D)
    s = None
    for r in rows:
        d = xT[r, cols] - mean
        t = jnp.sum((d * d).reshape(lm // 8, 8, n), axis=0)
        s = t if s is None else s + t
        if pin is not None:
            xnT[8:16, pin] = pltpu.bitcast(s, U32)
        yield
    rstd = lax.rsqrt(jnp.sum(s, axis=0, keepdims=True) * (1.0 / D) + 1e-5)
    for r in rows:
        _st(xnT, r, cols, ((xT[r, cols] - mean) * rstd).astype(BF16))
        yield


LM = cfg('LM', 32)
N_LN = 3 * D // LM


def _kernel(x_hbm, wa_hbm, wphi_ref, woa_hbm, wb_hbm, wob_hbm, out_ref,
            xs, wraw_a, wraw_b, wraw_o, tmp,
            xT, xnT, oT, wa_kv, wa_q, woT, wb,
            kvacc, zacc, zb, kvm, qbuf, kbuf, vbuf, sems):

    x_cp = [pltpu.make_async_copy(x_hbm.at[:, i * 128:(i + 1) * 128], xs.at[i], sems.at[i])
            for i in range(8)]

    def w_copies(gp):
        sem = sems.at[8 + gp]
        cps = []
        for part in (1, 2, 0):
            cols = pl.ds(pl.multiple_of(part * D + gp * 128, 128), 128)
            cps.append(pltpu.make_async_copy(wa_hbm.at[:, cols], wraw_a.at[:, cols], sem))
        for i in range(3):
            u = gp * 3 + i
            blk = (pl.ds(pl.multiple_of((u % 2) * 512, 512), 512),
                   pl.ds(pl.multiple_of((u // 2) * 256, 256), 256))
            cps.append(pltpu.make_async_copy(wb_hbm.at[blk], wraw_b.at[blk], sem))
        return cps

    wo_cp = [pltpu.make_async_copy(woa_hbm, wraw_o.at[0:D], sems.at[16]),
             pltpu.make_async_copy(wob_hbm, wraw_o.at[D:2 * D], sems.at[16])]
    for c in x_cp:
        c.start()
    for gp in range(8):
        for c in w_copies(gp):
            c.start()
    for c in wo_cp:
        c.start()

    xT[:, 0:PAD] = jnp.zeros((D, PAD), F32)
    zacc[7 * 256:8 * 256, :] = jnp.zeros((256, 128), F32)
    kvacc[7 * 128:8 * 128, :] = jnp.zeros((128, 128), F32)
    qbuf[...] = jnp.zeros(qbuf.shape, F32)
    kbuf[...] = jnp.zeros(kbuf.shape, F32)
    vbuf[...] = jnp.zeros(vbuf.shape, F32)

    for c in x_cp:
        c.wait()
    xu = xs.bitcast(U32)
    for r in range(8):
        for i in range(8):
            t = xu[i, pl.ds(r, 128, stride=8), :].T
            rows = slice(i * 128, (i + 1) * 128)
            xT[rows, PAD + r * 128:PAD + (r + 1) * 128] = pltpu.bitcast(t << 16, F32)
            xT[rows, PAD + 1024 + r * 128:PAD + 1024 + (r + 1) * 128] = pltpu.bitcast(
                t & jnp.uint32(0xFFFF0000), F32)
        for par in range(2):
            c0 = PAD + par * 1024 + r * 128
            _drain(_ln_pieces(xT, xnT, slice(c0, c0 + 128), 128))

    row = lax.broadcasted_iota(jnp.int32, (128, 128), 0)
    col = lax.broadcasted_iota(jnp.int32, (128, 128), 1)
    src_head = 2 * (row // 64) + row % 2
    src_j = (row % 64) // 2
    perm_h2 = ((src_head * 32 + src_j) == col).astype(BF16)
    sel_f = (lax.broadcasted_iota(jnp.int32, (128, 32), 0) % 64 // 2
             == lax.broadcasted_iota(jnp.int32, (128, 32), 1)).astype(BF16)

    def prep_a(blk):
        c0 = pl.multiple_of(blk * 128, 128)
        wphi = wphi_ref[pl.ds(c0, 128), :]
        fold = jnp.where(src_head == col // 32, _dot_nt(sel_f, wphi), 0.0).astype(BF16)
        k = (_dot_nt(fold, wraw_a[:, pl.ds(D + c0, 128)]) * LOG2E).astype(BF16)
        v = _dot_nt(perm_h2, wraw_a[:, pl.ds(2 * D + c0, 128)]).astype(BF16)
        q = _dot_nt(fold, wraw_a[:, pl.ds(c0, 128)]) * LOG2E
        r0 = pl.multiple_of(blk * 256, 256)
        _st(wa_kv, (r0, 64), slice(None), k[:64])
        _st(wa_kv, (r0 + 64, 64), slice(None), v[:64])
        _st(wa_kv, (r0 + 128, 64), slice(None), k[64:])
        _st(wa_kv, (r0 + 192, 64), slice(None), v[64:])
        _st(wa_q, (c0, 128), slice(None), q.astype(BF16))

    def prep_wb_pieces(gp):
        for i in range(3):
            u = gp * 3 + i
            kh, grp = u % 2, u // 2
            base = pl.multiple_of((grp % 4) * 384 + (grp // 4) * 128, 128)
            for half in range(2):
                w = wraw_b[pl.ds(pl.multiple_of(kh * 512, 512), 512),
                           pl.ds(pl.multiple_of(grp * 256 + half * 128, 128), 128)]
                t = w.astype(F32).T
                for j in range(2):
                    p = pltpu.pack_elementwise([t[64 * j:64 * j + 32], t[64 * j + 32:64 * j + 64]],
                                               packed_dtype=BF16)
                    for kt in range(4):
                        v = wb.at[kh * 4 + kt, pl.ds(base, 128), :]
                        v[pl.ds(half * 2 + j, 32, stride=4), :] = p[:, kt * 128:(kt + 1) * 128]
                yield

    def prep_wo_pieces(j):
        r0 = pl.multiple_of(j * 128, 128)
        for n in range(0, 8, 2):
            for i in range(n, n + 2):
                w = wraw_o[pl.ds(r0, 128), i * 128:(i + 1) * 128].astype(F32)
                p = jnp.concatenate(
                    [pltpu.pack_elementwise([w[64 * gl:64 * gl + 32], w[64 * gl + 32:64 * gl + 64]],
                                            packed_dtype=BF16) for gl in range(2)], axis=0)
                wp = pltpu.bitcast(p, BF16)
                _st(woT, slice(i * 128, (i + 1) * 128), pl.ds(r0, 128), wp.T, lead=(0,))
            yield
        hg, nh = j // 2, j % 2
        rb = pl.multiple_of(D + hg * 256, 256)
        for n in range(0, 4, 2):
            for i in range(n, n + 2):
                cols = pl.ds(pl.multiple_of(nh * 512 + i * 128, 128), 128)
                w = wraw_o[pl.ds(rb, 256), cols].astype(F32)
                for jj in range(4):
                    tmp[i, pl.ds(jj, 32, stride=4), :] = pltpu.pack_elementwise(
                        [w[64 * jj:64 * jj + 32], w[64 * jj + 32:64 * jj + 64]], packed_dtype=BF16)
            for i in range(n, n + 2):
                wp = pltpu.bitcast(tmp[i], BF16)
                _st(woT, (nh * 512 + i * 128, 128), pl.ds(pl.multiple_of(hg * 256, 256), 256),
                    wp.T, lead=(1,))
            yield

    N_PWO = 6
    N_PWB = 6

    def a_finalize_pieces(gp):
        for gl in range(2):
            g = gp * 2 + gl
            r0 = pl.multiple_of(g * 128, 128)
            z = jnp.sum(zacc[pl.ds(r0, 128), :], axis=1, keepdims=True)
            zb[pl.ds(r0, 128), :] = jnp.broadcast_to(z, (128, 128))
            r1 = pl.multiple_of(g * 64, 64)
            same = (lax.broadcasted_iota(jnp.int32, (64, 128), 0) % 2
                    == lax.broadcasted_iota(jnp.int32, (64, 128), 1) % 2)
            _st(kvm, (r1, 64), slice(None), jnp.where(same, kvacc[pl.ds(r1, 64), :], 0.0).astype(BF16))
            yield

    def kv_pieces(gp):
        seq = [(gl, c) for gl in range(2) for c in range(NCH)]
        pend = None
        kv = z = None
        for i in range(len(seq) + 1):
            res = None
            if i < len(seq):
                gl, c = seq[i]
                res = _dot(_ld(wa_kv, (gp * 256 + gl * 128, 128)),
                           _ld(xnT, slice(0, D), slice(PAD + c * NC, PAD + (c + 1) * NC)))
            if pend is not None:
                gl, c = seq[i - 1]
                a, b = _hedgehog(pend[:64])
                phi = jnp.concatenate([a, b], axis=0)
                zt = phi[:, :128] + phi[:, 128:]
                kt = _dot_nt(pend[64:].astype(BF16), phi.astype(BF16))
                z = zt if c == 0 else z + zt
                kv = kt if c == 0 else kv + kt
                if c == NCH - 1:
                    g = gp * 2 + gl
                    zacc[pl.ds(pl.multiple_of(g * 128, 128), 128), :] = z
                    kvacc[pl.ds(pl.multiple_of(g * 64, 64), 64), :] = kv
                wraw_b[D:D + 16, 0:128] = a[0:16, 0:128].astype(BF16)
                wb[0, 1536:1544, :] = pltpu.bitcast(a[0:8, 0:128], U32)
                yield
            pend = res

    def a_phase1(layer, gp, _):
        @pl.when(layer == 0)
        def _prep():
            for c in w_copies(gp):
                c.wait()
            prep_a(gp)

        _interleave(kv_pieces(gp), 2 * NCH, (prep_wb_pieces(gp), N_PWB),
                    (a_finalize_pieces((gp + 7) % 8), 2), lead=cfg("P1LEAD", 2))
        return _

    def q_pieces(j):
        cols = pl.ds(pl.multiple_of(j * NC, NC), NC)
        xcols = pl.ds(pl.multiple_of(PAD + j * NC, NC), NC)
        pq, pn = None, None
        for gg in range(18):
            res = None
            if gg < 16:
                res = _dot(_ld(wa_q, slice(gg * 64, (gg + 1) * 64)), _ld(xnT, slice(0, D), xcols))
            num = None
            res_done = False
            if pq is not None and gg - 1 < 16:
                g = gg - 1
                a, b = _hedgehog(pq)
                za = zb[g * 128:g * 128 + 64, :]
                zb_ = zb[g * 128 + 64:(g + 1) * 128, :]
                za = jnp.concatenate([za, za], axis=1)
                zb_ = jnp.concatenate([zb_, zb_], axis=1)
                den = _red_h2((a * za + b * zb_).reshape(8, 8, NC), jnp.add)
                inv = pl.reciprocal(den + 1e-6, approx=True)
                phi = jnp.concatenate([a, b], axis=0).astype(BF16)
                num = (_dot(_ld(kvm, slice(g * 64, (g + 1) * 64)), phi), inv)
                res_done, anchor = True, phi[0:16, 0:128]
            if pn is not None:
                g = gg - 2
                n_, inv_ = pn
                o = (n_.reshape(8, 8, NC) * inv_).reshape(64, NC)
                _st(oT, slice(g * 64, (g + 1) * 64), cols, o.astype(BF16))
                if not res_done:
                    res_done, anchor = True, o[0:16, 0:128].astype(BF16)
            pq, pn = res, num
            if res_done:
                wraw_o[2 * D:2 * D + 16, 0:128] = anchor
                woT[0, 512:520, 0:128] = pltpu.bitcast(anchor, U32)
                yield

    def a_phase2(layer, j, _):
        @pl.when(jnp.logical_and(layer == 0, j == 0))
        def _wait():
            for c in wo_cp:
                c.wait()

        _interleave(q_pieces(j), 17, (prep_wo_pieces(j), N_PWO), lead=cfg("P2LEAD", 2))
        return _

    def qkv_pieces(par, hg, slot):
        nm = 768 // QM
        per = 256 // QM
        def issue(n, m):
            xcols = pl.ds(pl.multiple_of(PAD + par * 1024 + n * NC, NC), NC)
            r0 = pl.multiple_of(hg * 768 + m * QM, QM)
            rp0 = pl.multiple_of(r0 // 2, QM // 2)
            w = jnp.concatenate([pltpu.bitcast(wb[kt, pl.ds(rp0, QM // 2), :], BF16) for kt in range(8)],
                                axis=1)
            return _dot(w, _ld(xnT, slice(0, D), xcols))
        def consume(n, m, res):
            rr = slice((m % per) * QM, (m % per) * QM + QM)
            if m < per:
                qbuf[slot, rr, n * NC:(n + 1) * NC] = res
            else:
                buf = kbuf if m < 2 * per else vbuf
                buf[slot, rr, 896 + n * NC:896 + (n + 1) * NC] = res
                for t in range(2 * n, 2 * n + 2):
                    if t >= 1:
                        sh = pltpu.roll(res[:, (t % 2) * 128:(t % 2) * 128 + 128], 1, 1)
                        buf[slot, rr, (t - 1) * 128:t * 128] = sh
            if cfg("BANCH", 0):
                oT[0:8, S:S + 128] = pltpu.bitcast(res[QM - 8:, NC - 128:], U32)
        seq = [(n, m) for n in range(4) for m in range(nm)]
        pend = None
        for i in range(len(seq) + QPIPE):
            if i < len(seq):
                res = issue(*seq[i])
            if not QPIPE:
                consume(*seq[i], res)
            elif pend is not None:
                consume(*seq[i - 1], pend)
            pend = res
            if i >= QPIPE:
                yield

    N_QKV = 4 * 768 // QM
    lane0 = lax.broadcasted_iota(jnp.int32, (8, 128), 1) == 0

    def attn_pieces(par, hg, slot):
        scale = DH ** -0.5 * LOG2E
        for rp in range(0, 8, 2):
            logit = [[None] * 8, [None] * 8]
            for dd in range(0, 32, 8):
                for d in range(dd, dd + 8):
                    rows = slice(d * 8, d * 8 + 8)
                    q = [qbuf[slot, rows, (rp + a) * 128:(rp + a + 1) * 128] for a in range(2)]
                    for e in range(rp, rp + 9):
                        k = kbuf[slot, rows, e * 128:(e + 1) * 128]
                        for a in range(2):
                            w = rp + a + 7 - e
                            if 0 <= w < 8:
                                t = q[a] * k
                                logit[a][w] = t if logit[a][w] is None else logit[a][w] + t
                yield
            prob = []
            for a in range(2):
                lg = []
                for w in range(8):
                    t = logit[a][w] * scale
                    if w > rp + a:
                        t = jnp.where(lane0, -1e9 * LOG2E, t)
                    lg.append(t)
                mx = functools.reduce(jnp.maximum, lg)
                ex = [jnp.exp2(t - mx) for t in lg]
                inv = pl.reciprocal(functools.reduce(jnp.add, ex), approx=True)
                prob.append([t * inv for t in ex])
            yield
            for dd in range(0, 32, 2):
                outs = []
                for d in (dd, dd + 1):
                    rows = slice(d * 8, d * 8 + 8)
                    acc = [None, None]
                    for e in range(rp, rp + 9):
                        v = vbuf[slot, rows, e * 128:(e + 1) * 128]
                        for a in range(2):
                            w = rp + a + 7 - e
                            if 0 <= w < 8:
                                t = prob[a][w] * v
                                acc[a] = t if acc[a] is None else acc[a] + t
                    outs.append(jnp.concatenate(acc, axis=1))
                o = jnp.concatenate(outs, axis=0).astype(BF16)
                r0 = pl.multiple_of(hg * 256 + dd * 8, 16)
                c0 = pl.multiple_of(par * 1024 + rp * 128, 256)
                _st(oT, (r0, 16), pl.ds(c0, 256), o)
                if dd % 8 == 6:
                    yield

    N_ATTN = 4 * 9

    def b_unit(i, _):
        prev = (i + 7) % 8
        _interleave(qkv_pieces(i // 4, i % 4, i % 2), N_QKV,
                    (attn_pieces(prev // 4, prev % 4, prev % 2), N_ATTN), lead=cfg("BLEAD", 2))
        return _

    def oproj_pieces(layer, cols, xv):
        for m in range(D // OM):
            rows = slice(m * OM, (m + 1) * OM)
            res = _dot(_ld(woT, rows, lead=(layer % 2,)), _ld(oT, slice(0, D), cols))
            xv[rows, NC:2 * NC] += res
            xnT[0:8, DUM:DUM + 128] = pltpu.bitcast(res[OM - 8:, NC - 128:], U32)
            xT[0:8, DUM:DUM + 128] = res[OM - 8:, NC - 128:]
            yield

    def o_chunk(layer, j, _):
        c0 = pl.multiple_of(j * NC, NC)
        xv = xT.at[:, pl.ds(c0, 2 * NC)]
        xnv = xnT.at[:, pl.ds(c0, 2 * NC)]
        _interleave(oproj_pieces(layer, pl.ds(c0, NC), xv), D // OM,
                    (_ln_pieces(xv, xnv, slice(0, NC), LM, pin=slice(NC, 2 * NC)), N_LN), lead=cfg("OLEAD", 2))
        return _

    ou = xs.bitcast(U32)

    def out_copy(m):
        cols = pl.ds(pl.multiple_of(m * 128, 128), 128)
        return pltpu.make_async_copy(xs.at[m], out_ref.at[:, cols], sems.at[m])

    def final_block(m, _):
        rows = pl.ds(pl.multiple_of(m * 128, 128), 128)
        w = _ld(woT, (m * 128, 128), lead=(1,))
        pend = None
        for r in range(9):
            res = None
            if r < 8:
                rhs = jnp.concatenate([_ld(oT, slice(0, D), slice(r * 128, (r + 1) * 128)),
                                       _ld(oT, slice(0, D), slice(1024 + r * 128, 1152 + r * 128))],
                                      axis=1)
                res = _dot(w, rhs)
            if pend is not None:
                c0 = PAD + (r - 1) * 128
                even = xT[rows, c0:c0 + 128] + pend[:, :128]
                odd = xT[rows, 1024 + c0:1152 + c0] + pend[:, 128:]
                word = pltpu.pack_elementwise([even, odd], packed_dtype=BF16)
                ou[m, pl.ds(r - 1, 128, stride=8), :] = word.T
            pend = res
        out_copy(m).start()
        return _

    def layer_body(layer, _):
        @pl.when(layer % 2 == 0)
        def _a():
            lax.fori_loop(0, 8, functools.partial(a_phase1, layer), None)
            _drain(a_finalize_pieces(7))
            lax.fori_loop(0, NCH, functools.partial(a_phase2, layer), None)

        @pl.when(layer % 2 == 1)
        def _b():
            lax.fori_loop(0, 8, b_unit, None)
            _drain(attn_pieces(1, 3, 1))

        @pl.when(layer < 3)
        def _o():
            lax.fori_loop(0, NCH, functools.partial(o_chunk, layer), None)
            _drain(_ln_pieces(xT, xnT, slice(S, S + PAD), 128))

        return _

    lax.fori_loop(0, 4, layer_body, None)
    lax.fori_loop(0, 8, final_block, None)
    for m in range(8):
        out_copy(m).wait()


@jax.jit
def pallas_interleave_layers__linear_kernel_hedgehog__sliding_local_dilated__prompt_kernel(
    A_x: jax.Array,
    A_wqkv: jax.Array,
    A_w_phi: jax.Array,
    A_wo: jax.Array,
    B_x: jax.Array,
    B_wqkv: jax.Array,
    B_wo: jax.Array,
):
    del B_x
    hbm = pl.BlockSpec(memory_space=pl.ANY)
    out = pl.pallas_call(
        _kernel,
        out_shape=jax.ShapeDtypeStruct((S, D), BF16),
        in_specs=[hbm, hbm, pl.BlockSpec(memory_space=pltpu.VMEM), hbm, hbm, hbm],
        out_specs=hbm,
        scratch_shapes=[
            pltpu.VMEM((8, S, 128), BF16),
            pltpu.VMEM((D, 3 * D), BF16),
            pltpu.VMEM((D + 16, 3 * D), BF16),
            pltpu.VMEM((2 * D + 16, D), BF16),
            pltpu.VMEM((4, 128, 128), U32),
            pltpu.VMEM((D, PAD + S + 128), F32),
            pltpu.VMEM((D // 2, PAD + S + 128), U32),
            pltpu.VMEM((D // 2, S + 128), U32),
            pltpu.VMEM((D, D), U32),
            pltpu.VMEM((D // 2, D), U32),
            pltpu.VMEM((2, D // 2 + 8, D), U32),
            pltpu.VMEM((8, 3 * D // 2 + 8, 128), U32),
            pltpu.VMEM((D, 128), F32),
            pltpu.VMEM((2 * D, 128), F32),
            pltpu.VMEM((2 * D, 128), F32),
            pltpu.VMEM((D // 2, 128), U32),
            pltpu.VMEM((2, 256, 1024), F32),
            pltpu.VMEM((2, 256, 1920), F32),
            pltpu.VMEM((2, 256, 1920), F32),
            pltpu.SemaphoreType.DMA((17,)),
        ],
        compiler_params=pltpu.CompilerParams(vmem_limit_bytes=110 * 2**20),
    )(A_x.reshape(S, D), A_wqkv, A_w_phi.reshape(H * DH, DH), A_wo, B_wqkv, B_wo)
    return out.reshape(1, S, D)
```

```python
import functools

import jax
import jax.numpy as jnp
from jax import lax
import jax.experimental.pallas as pl
import jax.experimental.pallas.tpu as pltpu

F32, BF16, U32 = jnp.float32, jnp.bfloat16, jnp.uint32
S, D, H, DH = 2048, 1024, 32, 32
NT = S // 128
NC = 256
NCH = S // NC
LOG2E = 1.4426950408889634
KOFF, VOFF, QDUM = 1024, 1024 + 1920, 1024 + 2 * 1920
PAD = NC
DUM = PAD + S
CFG = {}
def cfg(k, d): return CFG.get(k, d)
OM = cfg("OM", 128)
OPIPE = cfg("OPIPE", 0)
QM = cfg("QM", 128)
LM = cfg("LM", 64)
QPIPE = cfg("QPIPE", 0)
NT_DIMS = (((1,), (1,)), ((), ()))


def _dot(a, b):
    return jnp.dot(a, b, preferred_element_type=F32)


def _dot_nt(a, b):
    return lax.dot_general(a, b, NT_DIMS, preferred_element_type=F32)


def _ld(ref, rows, cols=slice(0, D), lead=()):
    if isinstance(rows, slice):
        a = rows.start or 0
        rows = slice(a // 2, None if rows.stop is None else rows.stop // 2)
    else:
        start, size = rows
        rows = pl.ds(pl.multiple_of(start // 2, 8), size // 2)
    return pltpu.bitcast(ref[lead + (rows, cols)], BF16)


def _st(ref, rows, cols, val, lead=()):
    if isinstance(rows, slice):
        rows = slice(rows.start // 2, rows.stop // 2)
    else:
        start, size = rows
        rows = pl.ds(pl.multiple_of(start // 2, 8), size // 2)
    ref[lead + (rows, cols)] = pltpu.bitcast(val, U32)


def _interleave(main, n_main, *sides, lead=0):
    done = [0] * len(sides)
    for i in range(n_main):
        next(main)
        for k, (g, n) in enumerate(sides):
            while done[k] < min(n, (i + 1) * n // (n_main - lead)):
                next(g)
                done[k] += 1
    for g in (main,) + tuple(g for g, _ in sides):
        for _ in g:
            raise AssertionError("generator piece count mismatch")


def _loop(n, body, unroll=1):
    def group(i, _):
        for u in range(unroll):
            body(i * unroll + u, None)
        return _
    lax.fori_loop(0, n // unroll, group, None)


def _drain(g):
    for _ in g:
        pass


def _red_h2(x, op):
    r = op(x[0], x[1])
    for i in range(2, 8):
        r = op(r, x[i])
    r = op(r, pltpu.roll(r, 4, 0))
    r = op(r, pltpu.roll(r, 2, 0))
    return r[None]


def _hedgehog(p):
    n = p.shape[1]
    p3 = p.reshape(8, 8, n)
    mx = _red_h2(p3, jnp.maximum)
    mn = _red_h2(p3, jnp.minimum)
    e1 = jnp.exp2(p3 - mx)
    e2 = jnp.exp2(mn - p3)
    s1 = _red_h2(e1, jnp.add)
    s2 = _red_h2(e2, jnp.add)
    a = (e1 * pl.reciprocal(s1, approx=True)).reshape(64, n)
    b = (e2 * pl.reciprocal(s2, approx=True)).reshape(64, n)
    return a, b


def _normalize_pieces(xT, xnT, cols, lm, s1, s2):
    mean = jnp.sum(s1, axis=0, keepdims=True) * (1.0 / D)
    var = jnp.maximum(jnp.sum(s2, axis=0, keepdims=True) * (1.0 / D) - mean * mean, 0.0)
    rstd = lax.rsqrt(var + 1e-5)
    for m in range(D // lm):
        r = slice(m * lm, (m + 1) * lm)
        _st(xnT, r, cols, ((xT[r, cols] - mean) * rstd).astype(BF16))
        yield


def _kernel(x_hbm, wa_hbm, wphi_ref, woa_hbm, wb_hbm, wob_hbm, out_ref,
            xs, wraw_a, wraw_b, wraw_o, tmp,
            xT, xnT, oT, wa_kv, wa_q, woT, wb,
            kvacc, zacc, zb, kvm, carry, carry_inv, stat, folds, qbuf, kbuf, vbuf, sems):

    x_cp = [pltpu.make_async_copy(x_hbm.at[:, i * 128:(i + 1) * 128], xs.at[i], sems.at[i])
            for i in range(8)]

    def w_copies(gp):
        sem = sems.at[8 + gp]
        cps = []
        for part in (1, 2, 0):
            cols = pl.ds(pl.multiple_of(part * D + gp * 128, 128), 128)
            cps.append(pltpu.make_async_copy(wa_hbm.at[:, cols], wraw_a.at[:, cols], sem))
        for i in range(3):
            u = gp * 3 + i
            blk = (pl.ds(pl.multiple_of((u % 2) * 512, 512), 512),
                   pl.ds(pl.multiple_of((u // 2) * 256, 256), 256))
            cps.append(pltpu.make_async_copy(wb_hbm.at[blk], wraw_b.at[blk], sem))
        return cps

    wo_cp = [pltpu.make_async_copy(woa_hbm, wraw_o.at[0:D], sems.at[16]),
             pltpu.make_async_copy(wob_hbm, wraw_o.at[D:2 * D], sems.at[16])]
    for c in x_cp:
        c.start()
    def start_w():
        for gp in range(8):
            for c in w_copies(gp):
                c.start()
        for c in wo_cp:
            c.start()

    if not cfg("WLATE", 0):
        start_w()

    xT[:, 0:PAD] = jnp.zeros((D, PAD), F32)
    carry[...] = jnp.zeros(carry.shape, F32)
    carry_inv[...] = jnp.zeros(carry_inv.shape, F32)
    stat[...] = jnp.zeros(stat.shape, F32)
    zacc[7 * 256:8 * 256, :] = jnp.zeros((256, 128), F32)
    kvacc[7 * 128:8 * 128, :] = jnp.zeros((128, 128), F32)
    qbuf[...] = jnp.zeros(qbuf.shape, F32)
    kbuf[...] = jnp.zeros(kbuf.shape, F32)
    vbuf[...] = jnp.zeros(vbuf.shape, F32)

    row = lax.broadcasted_iota(jnp.int32, (128, 128), 0)
    col = lax.broadcasted_iota(jnp.int32, (128, 128), 1)
    src_head = 2 * (row // 64) + row % 2
    src_j = (row % 64) // 2
    perm_h2 = ((src_head * 32 + src_j) == col).astype(BF16)
    sel_f = (lax.broadcasted_iota(jnp.int32, (128, 32), 0) % 64 // 2
             == lax.broadcasted_iota(jnp.int32, (128, 32), 1)).astype(BF16)

    def make_fold(blk, _):
        c0 = pl.multiple_of(blk * 128, 128)
        wphi = wphi_ref[pl.ds(c0, 128), :]
        fold = jnp.where(src_head == col // 32, _dot_nt(sel_f, wphi), 0.0).astype(BF16)
        _st(folds, (c0, 128), slice(0, 128), fold)
        return _

    lax.fori_loop(0, 8, make_fold, None)

    for c in x_cp:
        c.wait()
    if cfg("WLATE", 0):
        start_w()
    def x_prep():
        xu = xs.bitcast(U32)
        for r in range(8):
            sums = [None] * 4
            for i in range(8):
                t = xu[i, pl.ds(r, 128, stride=8), :].T
                halves = (pltpu.bitcast(t << 16, F32), pltpu.bitcast(t & jnp.uint32(0xFFFF0000), F32))
                for par, v in enumerate(halves):
                    c0 = PAD + par * 1024 + r * 128
                    xT[i * 128:(i + 1) * 128, c0:c0 + 128] = v
                    for k, u in enumerate((v, v * v)):
                        u = jnp.sum(u.reshape(16, 8, 128), axis=0)
                        sums[2 * par + k] = u if i == 0 else sums[2 * par + k] + u
            for par in range(2):
                c0 = PAD + par * 1024 + r * 128
                _drain(_normalize_pieces(xT, xnT, slice(c0, c0 + 128), 128, *sums[2 * par:2 * par + 2]))

    x_prep()

    def prep_a(blk):
        c0 = pl.multiple_of(blk * 128, 128)
        fold = _ld(folds, (c0, 128), slice(0, 128))
        k = (_dot_nt(fold, wraw_a[:, pl.ds(D + c0, 128)]) * LOG2E).astype(BF16)
        v = _dot_nt(perm_h2, wraw_a[:, pl.ds(2 * D + c0, 128)]).astype(BF16)
        q = _dot_nt(fold, wraw_a[:, pl.ds(c0, 128)]) * LOG2E
        r0 = pl.multiple_of(blk * 256, 256)
        _st(wa_kv, (r0, 64), slice(0, D), k[:64])
        _st(wa_kv, (r0 + 64, 64), slice(0, D), v[:64])
        _st(wa_kv, (r0 + 128, 64), slice(0, D), k[64:])
        _st(wa_kv, (r0 + 192, 64), slice(0, D), v[64:])
        _st(wa_q, (c0, 128), slice(0, D), q.astype(BF16))

    def prep_wb_pieces(gp):
        for i in range(3):
            u = gp * 3 + i
            kh, grp = u % 2, u // 2
            base = pl.multiple_of((grp % 4) * 384 + (grp // 4) * 128, 128)
            for half in range(2):
                w = wraw_b[pl.ds(pl.multiple_of(kh * 512, 512), 512),
                           pl.ds(pl.multiple_of(grp * 256 + half * 128, 128), 128)]
                t = w.astype(F32).T
                for j in range(2):
                    p = pltpu.pack_elementwise([t[64 * j:64 * j + 32], t[64 * j + 32:64 * j + 64]],
                                               packed_dtype=BF16)
                    for kt in range(4):
                        v = wb.at[kh * 4 + kt, pl.ds(base, 128), :]
                        v[pl.ds(half * 2 + j, 32, stride=4), :] = p[:, kt * 128:(kt + 1) * 128]
                yield

    def prep_wo_pieces(j):
        r0 = pl.multiple_of(j * 128, 128)
        for n in range(0, 8, 2):
            for i in range(n, n + 2):
                w = wraw_o[pl.ds(r0, 128), i * 128:(i + 1) * 128].astype(F32)
                p = jnp.concatenate(
                    [pltpu.pack_elementwise([w[64 * gl:64 * gl + 32], w[64 * gl + 32:64 * gl + 64]],
                                            packed_dtype=BF16) for gl in range(2)], axis=0)
                wp = pltpu.bitcast(p, BF16)
                _st(woT, slice(i * 128, (i + 1) * 128), pl.ds(r0, 128), wp.T, lead=(0,))
            yield
        hg, nh = j // 2, j % 2
        rb = pl.multiple_of(D + hg * 256, 256)
        for n in range(0, 4, 2):
            for i in range(n, n + 2):
                cols = pl.ds(pl.multiple_of(nh * 512 + i * 128, 128), 128)
                w = wraw_o[pl.ds(rb, 256), cols].astype(F32)
                for jj in range(4):
                    tmp[i, pl.ds(jj, 32, stride=4), :] = pltpu.pack_elementwise(
                        [w[64 * jj:64 * jj + 32], w[64 * jj + 32:64 * jj + 64]], packed_dtype=BF16)
            for i in range(n, n + 2):
                wp = pltpu.bitcast(tmp[i], BF16)
                _st(woT, (nh * 512 + i * 128, 128), pl.ds(pl.multiple_of(hg * 256, 256), 256),
                    wp.T, lead=(1,))
            yield

    N_PWO = 6
    N_PWB = 6

    def a_finalize_pieces(gp):
        for gl in range(2):
            g = gp * 2 + gl
            r0 = pl.multiple_of(g * 128, 128)
            z = jnp.sum(zacc[pl.ds(r0, 128), :], axis=1, keepdims=True)
            zb[pl.ds(r0, 128), :] = jnp.broadcast_to(z, (128, 128))
            r1 = pl.multiple_of(g * 64, 64)
            same = (lax.broadcasted_iota(jnp.int32, (64, 128), 0) % 2
                    == lax.broadcasted_iota(jnp.int32, (64, 128), 1) % 2)
            _st(kvm, (r1, 64), slice(None), jnp.where(same, kvacc[pl.ds(r1, 64), :], 0.0).astype(BF16))
            yield

    def kv_epilogue(res):
        a, b = _hedgehog(res[:64])
        phi = jnp.concatenate([a, b], axis=0)
        zt = phi[:, :128] + phi[:, 128:]
        kt = _dot_nt(res[64:].astype(BF16), phi.astype(BF16))
        return zt, kt, a

    def kv_tail(gp):
        zt, kt, a = kv_epilogue(carry[...])
        g = gp * 2 + 1
        zacc[pl.ds(pl.multiple_of(g * 128, 128), 128), :] += zt
        kvacc[pl.ds(pl.multiple_of(g * 64, 64), 64), :] += kt
        return a

    def kv_pieces(gp):
        seq = [(gl, c) for gl in range(2) for c in range(NCH)]
        pend = None
        kv = z = None
        for i in range(len(seq)):
            gl, c = seq[i]
            res = _dot(_ld(wa_kv, (gp * 256 + gl * 128, 128)),
                       _ld(xnT, slice(0, D), slice(PAD + c * NC, PAD + (c + 1) * NC)))
            if pend is None:
                a = kv_tail((gp + 7) % 8)
            else:
                gl, c = seq[i - 1]
                zt, kt, a = kv_epilogue(pend)
                z = zt if c == 0 else z + zt
                kv = kt if c == 0 else kv + kt
                if c == NCH - 1 or i == len(seq) - 1:
                    g = gp * 2 + gl
                    zacc[pl.ds(pl.multiple_of(g * 128, 128), 128), :] = z
                    kvacc[pl.ds(pl.multiple_of(g * 64, 64), 64), :] = kv
            wraw_b[D:D + 16, 0:128] = a[0:16, 0:128].astype(BF16)
            wb[0, 1536:1544, :] = pltpu.bitcast(a[0:8, 0:128], U32)
            yield
            pend = res
        carry[...] = pend

    def a_phase1(layer, n, i, _):
        @pl.when(layer == 0)
        def _prep():
            for u in range(n):
                for c in w_copies(i * n + u):
                    c.wait()
                prep_a(i * n + u)

        for u in range(n):
            gp = i * n + u
            _interleave(kv_pieces(gp), 2 * NCH, (prep_wb_pieces(gp), N_PWB),
                        (a_finalize_pieces((gp + 7) % 8), 2), lead=cfg("P1LEAD", 1))
        return _

    def q_features(g, pq):
        a, b = _hedgehog(pq)
        za = zb[g * 128:g * 128 + 64, :]
        zn = zb[g * 128 + 64:(g + 1) * 128, :]
        za = jnp.concatenate([za, za], axis=1)
        zn = jnp.concatenate([zn, zn], axis=1)
        den = _red_h2((a * za + b * zn).reshape(8, 8, NC), jnp.add)
        inv = pl.reciprocal(den + 1e-6, approx=True)
        phi = jnp.concatenate([a, b], axis=0).astype(BF16)
        return _dot(_ld(kvm, slice(g * 64, (g + 1) * 64), slice(0, 128)), phi), inv, phi

    def q_store(g, cols, num, inv):
        o = (num.reshape(8, 8, NC) * inv).reshape(64, NC)
        _st(oT, slice(g * 64, (g + 1) * 64), cols, o.astype(BF16))

    def q_pieces(j):
        cols = pl.ds(pl.multiple_of(j * NC, NC), NC)
        pcols = pl.ds(pl.multiple_of(((j + NCH - 1) % NCH) * NC, NC), NC)
        xcols = pl.ds(pl.multiple_of(PAD + j * NC, NC), NC)
        pq = carry[0:64]
        pn = (carry[64:128], carry_inv[...][None])
        for g in range(16):
            res = _dot(_ld(wa_q, slice(g * 64, (g + 1) * 64)), _ld(xnT, slice(0, D), xcols))
            num, inv, phi = q_features((g + 15) % 16, pq)
            q_store((g + 14) % 16, cols if g >= 2 else pcols, *pn)
            pq, pn = res, (num, inv)
            anchor = phi[0:16, 0:128]
            wraw_o[2 * D:2 * D + 16, 0:128] = anchor
            woT[0, 512:520, 0:128] = pltpu.bitcast(anchor, U32)
            yield
        carry[0:64] = pq
        carry[64:128] = pn[0]
        carry_inv[...] = pn[1][0]

    def q_tail():
        cols = slice(S - NC, S)
        num, inv, _phi = q_features(15, carry[0:64])
        q_store(14, cols, carry[64:128], carry_inv[...][None])
        q_store(15, cols, num, inv)

    def a_phase2(j, _):
        _interleave(q_pieces(j), 16, (prep_wo_pieces(j), N_PWO), lead=cfg("P2LEAD", 2))
        return _

    def qkv_pieces(par, hg, slot):
        nm = 768 // QM
        per = 256 // QM
        def issue(n, m):
            xcols = pl.ds(pl.multiple_of(PAD + par * 1024 + n * NC, NC), NC)
            r0 = pl.multiple_of(hg * 768 + m * QM, QM)
            rp0 = pl.multiple_of(r0 // 2, QM // 2)
            w = jnp.concatenate([pltpu.bitcast(wb[kt, pl.ds(rp0, QM // 2), :], BF16) for kt in range(8)],
                                axis=1)
            return _dot(w, _ld(xnT, slice(0, D), xcols))
        def consume(n, m, res):
            rr = slice((m % per) * QM, (m % per) * QM + QM)
            if m < per:
                qbuf[slot, rr, n * NC:(n + 1) * NC] = res
            else:
                buf = kbuf if m < 2 * per else vbuf
                buf[slot, rr, 896 + n * NC:896 + (n + 1) * NC] = res
                for t in range(2 * n, 2 * n + 2):
                    if t >= 1:
                        sh = pltpu.roll(res[:, (t % 2) * 128:(t % 2) * 128 + 128], 1, 1)
                        buf[slot, rr, (t - 1) * 128:t * 128] = sh
            if cfg("BANCH", 0):
                oT[0:8, S:S + 128] = pltpu.bitcast(res[QM - 8:, NC - 128:], U32)
        seq = [(n, m) for n in range(4) for m in range(nm)]
        pend = None
        for i in range(len(seq) + QPIPE):
            if i < len(seq):
                res = issue(*seq[i])
            if not QPIPE:
                consume(*seq[i], res)
            elif pend is not None:
                consume(*seq[i - 1], pend)
            pend = res
            if i >= QPIPE:
                yield

    N_QKV = 4 * 768 // QM
    lane0 = lax.broadcasted_iota(jnp.int32, (8, 128), 1) == 0

    def attn_pieces(par, hg, slot):
        scale = DH ** -0.5 * LOG2E
        for rp in range(0, 8, 2):
            logit = [[None] * 8, [None] * 8]
            for dd in range(0, 32, 8):
                for d in range(dd, dd + 8):
                    rows = slice(d * 8, d * 8 + 8)
                    q = [qbuf[slot, rows, (rp + a) * 128:(rp + a + 1) * 128] for a in range(2)]
                    for e in range(rp, rp + 9):
                        k = kbuf[slot, rows, e * 128:(e + 1) * 128]
                        for a in range(2):
                            w = rp + a + 7 - e
                            if 0 <= w < 8:
                                t = q[a] * k
                                logit[a][w] = t if logit[a][w] is None else logit[a][w] + t
                yield
            prob = []
            for a in range(2):
                lg = []
                for w in range(8):
                    t = logit[a][w] * scale
                    if w > rp + a:
                        t = jnp.where(lane0, -1e9 * LOG2E, t)
                    lg.append(t)
                mx = functools.reduce(jnp.maximum, lg)
                ex = [jnp.exp2(t - mx) for t in lg]
                inv = pl.reciprocal(functools.reduce(jnp.add, ex), approx=True)
                prob.append([t * inv for t in ex])
            yield
            for dd in range(0, 32, 2):
                outs = []
                for d in (dd, dd + 1):
                    rows = slice(d * 8, d * 8 + 8)
                    acc = [None, None]
                    for e in range(rp, rp + 9):
                        v = vbuf[slot, rows, e * 128:(e + 1) * 128]
                        for a in range(2):
                            w = rp + a + 7 - e
                            if 0 <= w < 8:
                                t = prob[a][w] * v
                                acc[a] = t if acc[a] is None else acc[a] + t
                    outs.append(jnp.concatenate(acc, axis=1))
                o = jnp.concatenate(outs, axis=0).astype(BF16)
                r0 = pl.multiple_of(hg * 256 + dd * 8, 16)
                c0 = pl.multiple_of(par * 1024 + rp * 128, 256)
                _st(oT, (r0, 16), pl.ds(c0, 256), o)
                if dd % 8 == 6:
                    yield

    N_ATTN = 4 * 9

    def b_unit(i, _):
        prev = (i + 7) % 8
        _interleave(qkv_pieces(i // 4, i % 4, i % 2), N_QKV,
                    (attn_pieces(prev // 4, prev % 4, prev % 2), N_ATTN), lead=cfg("BLEAD", 2))
        return _

    def oproj_pieces(layer, cols, xv):
        s1 = s2 = None
        for m in range(D // OM):
            rows = slice(m * OM, (m + 1) * OM)
            res = _dot(_ld(woT, rows, lead=(layer % 2,)), _ld(oT, slice(0, D), cols))
            x = xv[rows, NC:2 * NC] + res
            xv[rows, NC:2 * NC] = x
            t1 = jnp.sum(x.reshape(OM // 8, 8, NC), axis=0)
            t2 = jnp.sum((x * x).reshape(OM // 8, 8, NC), axis=0)
            s1, s2 = (t1, t2) if m == 0 else (s1 + t1, s2 + t2)
            xnT[0:8, DUM:DUM + 128] = pltpu.bitcast(res[OM - 8:, NC - 128:], U32)
            xT[0:8, DUM:DUM + 128] = res[OM - 8:, NC - 128:]
            yield
        stat[0] = s1
        stat[1] = s2

    def o_chunk(layer, j, _):
        c0 = pl.multiple_of(j * NC, NC)
        xv = xT.at[:, pl.ds(c0, 2 * NC)]
        xnv = xnT.at[:, pl.ds(c0, 2 * NC)]
        _interleave(oproj_pieces(layer, pl.ds(c0, NC), xv), D // OM,
                    (_normalize_pieces(xv, xnv, slice(0, NC), LM, stat[0], stat[1]), D // LM),
                    lead=cfg("OLEAD", 1))
        return _

    ou = xs.bitcast(U32)

    def out_copy(m):
        cols = pl.ds(pl.multiple_of(m * 128, 128), 128)
        return pltpu.make_async_copy(xs.at[m], out_ref.at[:, cols], sems.at[m])

    def final_block(m, _):
        rows = pl.ds(pl.multiple_of(m * 128, 128), 128)
        w = _ld(woT, (m * 128, 128), lead=(1,))
        pend = None
        for r in range(9):
            res = None
            if r < 8:
                rhs = jnp.concatenate([_ld(oT, slice(0, D), slice(r * 128, (r + 1) * 128)),
                                       _ld(oT, slice(0, D), slice(1024 + r * 128, 1152 + r * 128))],
                                      axis=1)
                res = _dot(w, rhs)
            if pend is not None:
                c0 = PAD + (r - 1) * 128
                even = xT[rows, c0:c0 + 128] + pend[:, :128]
                odd = xT[rows, 1024 + c0:1152 + c0] + pend[:, 128:]
                word = pltpu.pack_elementwise([even, odd], packed_dtype=BF16)
                ou[m, pl.ds(r - 1, 128, stride=8), :] = word.T
            pend = res
        out_copy(m).start()
        return _

    def layer_body(layer, _):
        @pl.when(layer % 2 == 0)
        def _a():
            lax.fori_loop(0, 8 // cfg('U1', 1), functools.partial(a_phase1, layer, cfg('U1', 1)), None)
            kv_tail(7)
            _drain(a_finalize_pieces(7))

            @pl.when(layer == 0)
            def _wait():
                for c in wo_cp:
                    c.wait()

            _loop(NCH, a_phase2, cfg('U2', 1))
            q_tail()

        @pl.when(layer % 2 == 1)
        def _b():
            _loop(8, b_unit, cfg('UB', 1))
            _drain(attn_pieces(1, 3, 1))

        @pl.when(layer < 3)
        def _o():
            _loop(NCH, functools.partial(o_chunk, layer), cfg('UO', 1))
            _drain(_normalize_pieces(xT, xnT, slice(S, S + PAD), 128, stat[0], stat[1]))

        return _

    lax.fori_loop(0, 4, layer_body, None)
    _loop(8, final_block, cfg('UF', 1))
    for m in range(8):
        out_copy(m).wait()


@jax.jit
def pallas_interleave_layers__linear_kernel_hedgehog__sliding_local_dilated__prompt_kernel(
    A_x: jax.Array,
    A_wqkv: jax.Array,
    A_w_phi: jax.Array,
    A_wo: jax.Array,
    B_x: jax.Array,
    B_wqkv: jax.Array,
    B_wo: jax.Array,
):
    del B_x
    hbm = pl.BlockSpec(memory_space=pl.ANY)
    out = pl.pallas_call(
        _kernel,
        out_shape=jax.ShapeDtypeStruct((S, D), BF16),
        in_specs=[hbm, hbm, pl.BlockSpec(memory_space=pltpu.VMEM), hbm, hbm, hbm],
        out_specs=hbm,
        scratch_shapes=[
            pltpu.VMEM((8, S, 128), BF16),
            pltpu.VMEM((D, 3 * D), BF16),
            pltpu.VMEM((D + 16, 3 * D), BF16),
            pltpu.VMEM((2 * D + 16, D), BF16),
            pltpu.VMEM((4, 128, 128), U32),
            pltpu.VMEM((D, PAD + S + 128), F32),
            pltpu.VMEM((D // 2, PAD + S + 128), U32),
            pltpu.VMEM((D // 2, S + 128), U32),
            pltpu.VMEM((D, D + cfg('WPAD', 0)), U32),
            pltpu.VMEM((D // 2, D + cfg('WPAD', 0)), U32),
            pltpu.VMEM((2, D // 2 + 8, D + cfg('WPAD', 0)), U32),
            pltpu.VMEM((8, 3 * D // 2 + 8, 128), U32),
            pltpu.VMEM((D, 128), F32),
            pltpu.VMEM((2 * D, 128), F32),
            pltpu.VMEM((2 * D, 128), F32),
            pltpu.VMEM((D // 2, 128), U32),
            pltpu.VMEM((128, NC), F32),
            pltpu.VMEM((8, NC), F32),
            pltpu.VMEM((2, 8, NC), F32),
            pltpu.VMEM((D // 2, 128), U32),
            pltpu.VMEM((2, 256, 1024 + cfg('QPAD', 128)), F32),
            pltpu.VMEM((2, 256, 1920), F32),
            pltpu.VMEM((2, 256, 1920), F32),
            pltpu.SemaphoreType.DMA((17,)),
        ],
        compiler_params=pltpu.CompilerParams(vmem_limit_bytes=110 * 2**20),
    )(A_x.reshape(S, D), A_wqkv, A_w_phi.reshape(H * DH, DH), A_wo, B_wqkv, B_wo)
    return out.reshape(1, S, D)
```

```python
import functools

import jax
import jax.numpy as jnp
from jax import lax
import jax.experimental.pallas as pl
import jax.experimental.pallas.tpu as pltpu

F32, BF16, U32 = jnp.float32, jnp.bfloat16, jnp.uint32
S, D, H, DH = 2048, 1024, 32, 32
NT = S // 128
NC = 256
NCH = S // NC
LOG2E = 1.4426950408889634
KOFF, VOFF, QDUM = 1024, 1024 + 1920, 1024 + 2 * 1920
PAD = NC
DUM = PAD + S
CFG = {}
def cfg(k, d): return CFG.get(k, d)
OM = cfg("OM", 128)
OPIPE = cfg("OPIPE", 0)
QM = cfg("QM", 256)
LM = cfg("LM", 64)
QPIPE = cfg("QPIPE", 0)
NT_DIMS = (((1,), (1,)), ((), ()))


def _dot(a, b):
    return jnp.dot(a, b, preferred_element_type=F32)


def _dot_nt(a, b):
    return lax.dot_general(a, b, NT_DIMS, preferred_element_type=F32)


def _ld(ref, rows, cols=slice(0, D), lead=()):
    if isinstance(rows, slice):
        a = rows.start or 0
        rows = slice(a // 2, None if rows.stop is None else rows.stop // 2)
    else:
        start, size = rows
        rows = pl.ds(pl.multiple_of(start // 2, 8), size // 2)
    return pltpu.bitcast(ref[lead + (rows, cols)], BF16)


def _st(ref, rows, cols, val, lead=()):
    if isinstance(rows, slice):
        rows = slice(rows.start // 2, rows.stop // 2)
    else:
        start, size = rows
        rows = pl.ds(pl.multiple_of(start // 2, 8), size // 2)
    ref[lead + (rows, cols)] = pltpu.bitcast(val, U32)


def _interleave(main, n_main, *sides, lead=0):
    done = [0] * len(sides)
    for i in range(n_main):
        next(main)
        for k, (g, n) in enumerate(sides):
            while done[k] < min(n, (i + 1) * n // (n_main - lead)):
                next(g)
                done[k] += 1
    for g in (main,) + tuple(g for g, _ in sides):
        for _ in g:
            raise AssertionError("generator piece count mismatch")


def _loop(n, body, unroll=1):
    def group(i, _):
        for u in range(unroll):
            body(i * unroll + u, None)
        return _
    lax.fori_loop(0, n // unroll, group, None)


def _drain(g):
    for _ in g:
        pass


def _red_h2(x, op):
    r = op(x[0], x[1])
    for i in range(2, 8):
        r = op(r, x[i])
    r = op(r, pltpu.roll(r, 4, 0))
    r = op(r, pltpu.roll(r, 2, 0))
    return r[None]


def _hedgehog(p):
    n = p.shape[1]
    p3 = p.reshape(8, 8, n)
    mx = _red_h2(p3, jnp.maximum)
    mn = _red_h2(p3, jnp.minimum)
    e1 = jnp.exp2(p3 - mx)
    e2 = jnp.exp2(mn - p3)
    s1 = _red_h2(e1, jnp.add)
    s2 = _red_h2(e2, jnp.add)
    a = (e1 * pl.reciprocal(s1, approx=True)).reshape(64, n)
    b = (e2 * pl.reciprocal(s2, approx=True)).reshape(64, n)
    return a, b


def _normalize_pieces(xT, xnT, cols, lm, s1, s2):
    mean = jnp.sum(s1, axis=0, keepdims=True) * (1.0 / D)
    var = jnp.maximum(jnp.sum(s2, axis=0, keepdims=True) * (1.0 / D) - mean * mean, 0.0)
    rstd = lax.rsqrt(var + 1e-5)
    for m in range(D // lm):
        r = slice(m * lm, (m + 1) * lm)
        _st(xnT, r, cols, ((xT[r, cols] - mean) * rstd).astype(BF16))
        yield


def _kernel(x_hbm, wa_hbm, wphi_ref, woa_hbm, wb_hbm, wob_hbm, out_ref,
            xs, wraw_a, wraw_b, wraw_o, tmp,
            xT, xnT, oT, wa_kv, wa_q, woT, wb,
            kvacc, zacc, zb, kvm, carry, carry_inv, stat, folds, qbuf, kbuf, vbuf, sems):

    x_cp = [pltpu.make_async_copy(x_hbm.at[:, i * 128:(i + 1) * 128], xs.at[i], sems.at[i])
            for i in range(8)]

    def w_copies(gp):
        sem = sems.at[8 + gp]
        cps = []
        for part in (1, 2, 0):
            cols = pl.ds(pl.multiple_of(part * D + gp * 128, 128), 128)
            cps.append(pltpu.make_async_copy(wa_hbm.at[:, cols], wraw_a.at[:, cols], sem))
        for i in range(3):
            u = gp * 3 + i
            blk = (pl.ds(pl.multiple_of((u % 2) * 512, 512), 512),
                   pl.ds(pl.multiple_of((u // 2) * 256, 256), 256))
            cps.append(pltpu.make_async_copy(wb_hbm.at[blk], wraw_b.at[blk], sem))
        return cps

    wo_cp = [pltpu.make_async_copy(woa_hbm, wraw_o.at[0:D], sems.at[16]),
             pltpu.make_async_copy(wob_hbm, wraw_o.at[D:2 * D], sems.at[16])]
    for c in x_cp:
        c.start()
    def start_w():
        for gp in range(8):
            for c in w_copies(gp):
                c.start()
        for c in wo_cp:
            c.start()

    if not cfg("WLATE", 0):
        start_w()

    xT[:, 0:PAD] = jnp.zeros((D, PAD), F32)
    carry[...] = jnp.zeros(carry.shape, F32)
    carry_inv[...] = jnp.zeros(carry_inv.shape, F32)
    stat[...] = jnp.zeros(stat.shape, F32)
    zacc[7 * 256:8 * 256, :] = jnp.zeros((256, 128), F32)
    kvacc[7 * 128:8 * 128, :] = jnp.zeros((128, 128), F32)
    def clear(i, _):
        rows = pl.ds(pl.multiple_of(i * 8, 8), 8)
        for buf in (qbuf, kbuf, vbuf):
            buf[1, rows, :] = jnp.zeros((8, buf.shape[2]), F32)
        return _
    lax.fori_loop(0, 32, clear, None)

    row = lax.broadcasted_iota(jnp.int32, (128, 128), 0)
    col = lax.broadcasted_iota(jnp.int32, (128, 128), 1)
    src_head = 2 * (row // 64) + row % 2
    src_j = (row % 64) // 2
    perm_h2 = ((src_head * 32 + src_j) == col).astype(BF16)
    sel_f = (lax.broadcasted_iota(jnp.int32, (128, 32), 0) % 64 // 2
             == lax.broadcasted_iota(jnp.int32, (128, 32), 1)).astype(BF16)

    def make_fold(blk, _):
        c0 = pl.multiple_of(blk * 128, 128)
        wphi = wphi_ref[pl.ds(c0, 128), :]
        fold = jnp.where(src_head == col // 32, _dot_nt(sel_f, wphi), 0.0).astype(BF16)
        _st(folds, (c0, 128), slice(0, 128), fold)
        return _

    lax.fori_loop(0, 8, make_fold, None)

    for c in x_cp:
        c.wait()
    if cfg("WLATE", 0):
        start_w()
    def x_prep():
        xu = xs.bitcast(U32)
        for r in range(8):
            sums = [None] * 4
            for i in range(8):
                t = xu[i, pl.ds(r, 128, stride=8), :].T
                halves = (pltpu.bitcast(t << 16, F32), pltpu.bitcast(t & jnp.uint32(0xFFFF0000), F32))
                for par, v in enumerate(halves):
                    c0 = PAD + par * 1024 + r * 128
                    xT[i * 128:(i + 1) * 128, c0:c0 + 128] = v
                    for k, u in enumerate((v, v * v)):
                        u = jnp.sum(u.reshape(16, 8, 128), axis=0)
                        sums[2 * par + k] = u if i == 0 else sums[2 * par + k] + u
            for par in range(2):
                c0 = PAD + par * 1024 + r * 128
                _drain(_normalize_pieces(xT, xnT, slice(c0, c0 + 128), 128, *sums[2 * par:2 * par + 2]))

    x_prep()

    def prep_a(blk):
        c0 = pl.multiple_of(blk * 128, 128)
        fold = _ld(folds, (c0, 128), slice(0, 128))
        k = (_dot_nt(fold, wraw_a[:, pl.ds(D + c0, 128)]) * LOG2E).astype(BF16)
        v = _dot_nt(perm_h2, wraw_a[:, pl.ds(2 * D + c0, 128)]).astype(BF16)
        q = _dot_nt(fold, wraw_a[:, pl.ds(c0, 128)]) * LOG2E
        r0 = pl.multiple_of(blk * 256, 256)
        _st(wa_kv, (r0, 64), slice(0, D), k[:64])
        _st(wa_kv, (r0 + 64, 64), slice(0, D), v[:64])
        _st(wa_kv, (r0 + 128, 64), slice(0, D), k[64:])
        _st(wa_kv, (r0 + 192, 64), slice(0, D), v[64:])
        _st(wa_q, (c0, 128), slice(0, D), q.astype(BF16))

    def prep_wb_pieces(gp):
        for i in range(3):
            u = gp * 3 + i
            kh, grp = u % 2, u // 2
            base = pl.multiple_of((grp % 4) * 384 + (grp // 4) * 128, 128)
            for half in range(2):
                w = wraw_b[pl.ds(pl.multiple_of(kh * 512, 512), 512),
                           pl.ds(pl.multiple_of(grp * 256 + half * 128, 128), 128)]
                t = w.astype(F32).T
                for j in range(2):
                    p = pltpu.pack_elementwise([t[64 * j:64 * j + 32], t[64 * j + 32:64 * j + 64]],
                                               packed_dtype=BF16)
                    for kt in range(4):
                        v = wb.at[kh * 4 + kt, pl.ds(base, 128), :]
                        v[pl.ds(half * 2 + j, 32, stride=4), :] = p[:, kt * 128:(kt + 1) * 128]
                yield

    def prep_wo_pieces(j):
        r0 = pl.multiple_of(j * 128, 128)
        for n in range(0, 8, WG):
            for i in range(n, n + WG):
                w = wraw_o[pl.ds(r0, 128), i * 128:(i + 1) * 128].astype(F32)
                p = jnp.concatenate(
                    [pltpu.pack_elementwise([w[64 * gl:64 * gl + 32], w[64 * gl + 32:64 * gl + 64]],
                                            packed_dtype=BF16) for gl in range(2)], axis=0)
                wp = pltpu.bitcast(p, BF16)
                _st(woT, slice(i * 128, (i + 1) * 128), pl.ds(r0, 128), wp.T, lead=(0,))
            yield
        hg, nh = j // 2, j % 2
        rb = pl.multiple_of(D + hg * 256, 256)
        for n in range(0, 4, WG):
            for i in range(n, n + WG):
                cols = pl.ds(pl.multiple_of(nh * 512 + i * 128, 128), 128)
                w = wraw_o[pl.ds(rb, 256), cols].astype(F32)
                for jj in range(4):
                    tmp[i, pl.ds(jj, 32, stride=4), :] = pltpu.pack_elementwise(
                        [w[64 * jj:64 * jj + 32], w[64 * jj + 32:64 * jj + 64]], packed_dtype=BF16)
            for i in range(n, n + WG):
                wp = pltpu.bitcast(tmp[i], BF16)
                _st(woT, (nh * 512 + i * 128, 128), pl.ds(pl.multiple_of(hg * 256, 256), 256),
                    wp.T, lead=(1,))
            yield

    WG = cfg('WG', 1)
    N_PWO = 12 // WG
    N_PWB = 6

    def a_finalize_pieces(gp):
        for gl in range(2):
            g = gp * 2 + gl
            r0 = pl.multiple_of(g * 128, 128)
            z = jnp.sum(zacc[pl.ds(r0, 128), :], axis=1, keepdims=True)
            zb[pl.ds(r0, 128), :] = jnp.broadcast_to(z, (128, 128))
            r1 = pl.multiple_of(g * 64, 64)
            same = (lax.broadcasted_iota(jnp.int32, (64, 128), 0) % 2
                    == lax.broadcasted_iota(jnp.int32, (64, 128), 1) % 2)
            _st(kvm, (r1, 64), slice(None), jnp.where(same, kvacc[pl.ds(r1, 64), :], 0.0).astype(BF16))
            yield

    def kv_epilogue(res):
        a, b = _hedgehog(res[:64])
        phi = jnp.concatenate([a, b], axis=0)
        zt = phi[:, :128] + phi[:, 128:]
        kt = _dot_nt(res[64:].astype(BF16), phi.astype(BF16))
        return zt, kt, a

    def kv_tail(gp):
        zt, kt, a = kv_epilogue(carry[0:128])
        g = gp * 2 + 1
        zacc[pl.ds(pl.multiple_of(g * 128, 128), 128), :] += zt
        kvacc[pl.ds(pl.multiple_of(g * 64, 64), 64), :] += kt
        return a

    def kv_pieces(gp):
        seq = [(gl, c) for gl in range(2) for c in range(NCH)]
        pend = None
        kv = z = None
        for i in range(len(seq)):
            gl, c = seq[i]
            res = _dot(_ld(wa_kv, (gp * 256 + gl * 128, 128)),
                       _ld(xnT, slice(0, D), slice(PAD + c * NC, PAD + (c + 1) * NC)))
            if pend is None:
                a = kv_tail((gp + 7) % 8)
            else:
                gl, c = seq[i - 1]
                zt, kt, a = kv_epilogue(pend)
                z = zt if c == 0 else z + zt
                kv = kt if c == 0 else kv + kt
                if c == NCH - 1 or i == len(seq) - 1:
                    g = gp * 2 + gl
                    zacc[pl.ds(pl.multiple_of(g * 128, 128), 128), :] = z
                    kvacc[pl.ds(pl.multiple_of(g * 64, 64), 64), :] = kv
            wraw_b[D:D + 16, 0:128] = a[0:16, 0:128].astype(BF16)
            wb[0, 1536:1544, :] = pltpu.bitcast(a[0:8, 0:128], U32)
            yield
            pend = res
        carry[0:128] = pend

    def a_phase1(layer, n, i, _):
        @pl.when(layer == 0)
        def _prep():
            for u in range(n):
                for c in w_copies(i * n + u):
                    c.wait()
                prep_a(i * n + u)

        for u in range(n):
            gp = i * n + u
            _interleave(kv_pieces(gp), 2 * NCH, (prep_wb_pieces(gp), N_PWB),
                        (a_finalize_pieces((gp + 7) % 8), 2), lead=cfg("P1LEAD", 1))
        return _

    def q_features(g, pq):
        a, b = _hedgehog(pq)
        za = zb[g * 128:g * 128 + 64, :]
        zn = zb[g * 128 + 64:(g + 1) * 128, :]
        za = jnp.concatenate([za, za], axis=1)
        zn = jnp.concatenate([zn, zn], axis=1)
        den = _red_h2((a * za + b * zn).reshape(8, 8, NC), jnp.add)
        inv = pl.reciprocal(den + 1e-6, approx=True)
        phi = jnp.concatenate([a, b], axis=0).astype(BF16)
        return _dot(_ld(kvm, slice(g * 64, (g + 1) * 64), slice(0, 128)), phi), inv, phi

    def q_store(g, cols, num, inv):
        o = (num.reshape(8, 8, NC) * inv).reshape(64, NC)
        _st(oT, slice(g * 64, (g + 1) * 64), cols, o.astype(BF16))

    GQ = cfg("GQ", 1)

    def q_pieces(j):
        cols = pl.ds(pl.multiple_of(j * NC, NC), NC)
        pcols = pl.ds(pl.multiple_of(((j + NCH - 1) % NCH) * NC, NC), NC)
        xcols = pl.ds(pl.multiple_of(PAD + j * NC, NC), NC)
        n = 64 * GQ
        pq = carry[0:n]
        pn = [(carry[n + 64 * t:n + 64 * (t + 1)], carry_inv[8 * t:8 * (t + 1)][None]) for t in range(GQ)]
        for g in range(0, 16, GQ):
            res = _dot(_ld(wa_q, slice(g * 64, g * 64 + n)), _ld(xnT, slice(0, D), xcols))
            new = []
            for t in range(GQ):
                num, inv, phi = q_features((g - GQ + t) % 16, pq[64 * t:64 * (t + 1)])
                q_store((g - 2 * GQ + t) % 16, cols if g >= 2 * GQ else pcols, *pn[t])
                new.append((num, inv))
            pq, pn = res, new
            anchor = phi[0:16, 0:128]
            wraw_o[2 * D:2 * D + 16, 0:128] = anchor
            woT[0, 512:520, 0:128] = pltpu.bitcast(anchor, U32)
            yield
        carry[0:n] = pq
        for t in range(GQ):
            carry[n + 64 * t:n + 64 * (t + 1)] = pn[t][0]
            carry_inv[8 * t:8 * (t + 1)] = pn[t][1][0]

    def q_tail():
        cols = slice(S - NC, S)
        n = 64 * GQ
        for t in range(GQ):
            num, inv, _phi = q_features(16 - GQ + t, carry[64 * t:64 * (t + 1)])
            q_store(16 - 2 * GQ + t, cols, carry[n + 64 * t:n + 64 * (t + 1)], carry_inv[8 * t:8 * (t + 1)][None])
            q_store(16 - GQ + t, cols, num, inv)

    def a_phase2(j, _):
        _interleave(q_pieces(j), 16 // GQ, (prep_wo_pieces(j), N_PWO), lead=cfg("P2LEAD", 4))
        return _

    QN = cfg("QN", 128)

    def qkv_pieces(par, hg, slot):
        per = 256 // QM
        for n in range(1024 // QN):
            xcols = pl.ds(pl.multiple_of(PAD + par * 1024 + n * QN, 128), QN)
            for m in range(3 * per):
                rp0 = pl.multiple_of(hg * 384 + m * (QM // 2), QM // 2)
                w = jnp.concatenate([pltpu.bitcast(wb[kt, pl.ds(rp0, QM // 2), :], BF16)
                                     for kt in range(8)], axis=1)
                res = _dot(w, _ld(xnT, slice(0, D), xcols))
                rr = slice((m % per) * QM, (m % per) * QM + QM)
                if m < per:
                    qbuf[slot, rr, n * QN:(n + 1) * QN] = res
                else:
                    buf = kbuf if m < 2 * per else vbuf
                    buf[slot, rr, 896 + n * QN:896 + (n + 1) * QN] = res
                    for i in range(QN // 128):
                        t = n * (QN // 128) + i
                        if t >= 1:
                            buf[slot, rr, (t - 1) * 128:t * 128] = pltpu.roll(
                                res[:, i * 128:(i + 1) * 128], 1, 1)
                yield

    N_QKV = (1024 // QN) * (768 // QM)
    lane0 = lax.broadcasted_iota(jnp.int32, (8, 128), 1) == 0

    def attn_pieces(par, hg, slot):
        scale = DH ** -0.5 * LOG2E
        for rp in range(0, 8, 2):
            logit = [[None] * 8, [None] * 8]
            for dd in range(0, 32, 8):
                for d in range(dd, dd + 8):
                    rows = slice(d * 8, d * 8 + 8)
                    q = [qbuf[slot, rows, (rp + a) * 128:(rp + a + 1) * 128] for a in range(2)]
                    for e in range(rp, rp + 9):
                        k = kbuf[slot, rows, e * 128:(e + 1) * 128]
                        for a in range(2):
                            w = rp + a + 7 - e
                            if 0 <= w < 8:
                                t = q[a] * k
                                logit[a][w] = t if logit[a][w] is None else logit[a][w] + t
                yield
            prob = []
            for a in range(2):
                lg = []
                for w in range(8):
                    t = logit[a][w] * scale
                    if w > rp + a:
                        t = jnp.where(lane0, -1e9 * LOG2E, t)
                    lg.append(t)
                mx = functools.reduce(jnp.maximum, lg)
                ex = [jnp.exp2(t - mx) for t in lg]
                inv = pl.reciprocal(functools.reduce(jnp.add, ex), approx=True)
                prob.append([t * inv for t in ex])
            yield
            for dd in range(0, 32, 2):
                outs = []
                for d in (dd, dd + 1):
                    rows = slice(d * 8, d * 8 + 8)
                    acc = [None, None]
                    for e in range(rp, rp + 9):
                        v = vbuf[slot, rows, e * 128:(e + 1) * 128]
                        for a in range(2):
                            w = rp + a + 7 - e
                            if 0 <= w < 8:
                                t = prob[a][w] * v
                                acc[a] = t if acc[a] is None else acc[a] + t
                    outs.append(jnp.concatenate(acc, axis=1))
                o = jnp.concatenate(outs, axis=0).astype(BF16)
                r0 = pl.multiple_of(hg * 256 + dd * 8, 16)
                c0 = pl.multiple_of(par * 1024 + rp * 128, 256)
                _st(oT, (r0, 16), pl.ds(c0, 256), o)
                if dd % 8 == 6:
                    yield

    N_ATTN = 4 * 9

    def b_unit(i, _):
        prev = (i + 7) % 8
        _interleave(qkv_pieces(i // 4, i % 4, i % 2), N_QKV,
                    (attn_pieces(prev // 4, prev % 4, prev % 2), N_ATTN), lead=cfg("BLEAD", 1))
        return _

    ON = cfg("ON", 256)

    def oproj_pieces(layer, c0, xv):
        for n in range(NC // ON):
            s1 = s2 = None
            xc = slice(NC + n * ON, NC + (n + 1) * ON)
            for m in range(D // OM):
                rows = slice(m * OM, (m + 1) * OM)
                res = _dot(_ld(woT, rows, lead=(layer % 2,)),
                           _ld(oT, slice(0, D), pl.ds(pl.multiple_of(c0 + n * ON, 128), ON)))
                x = xv[rows, xc] + res
                xv[rows, xc] = x
                t1 = jnp.sum(x.reshape(OM // 8, 8, ON), axis=0)
                t2 = jnp.sum((x * x).reshape(OM // 8, 8, ON), axis=0)
                s1, s2 = (t1, t2) if m == 0 else (s1 + t1, s2 + t2)
                xnT[0:8, DUM:DUM + 128] = pltpu.bitcast(res[OM - 8:, ON - 128:], U32)
                xT[0:8, DUM:DUM + 128] = res[OM - 8:, ON - 128:]
                yield
            stat[0, :, n * ON:(n + 1) * ON] = s1
            stat[1, :, n * ON:(n + 1) * ON] = s2

    def o_chunk(layer, j, _):
        c0 = pl.multiple_of(j * NC, NC)
        xv = xT.at[:, pl.ds(c0, 2 * NC)]
        xnv = xnT.at[:, pl.ds(c0, 2 * NC)]
        _interleave(oproj_pieces(layer, c0, xv), (D // OM) * (NC // ON),
                    (_normalize_pieces(xv, xnv, slice(0, NC), LM, stat[0], stat[1]), D // LM),
                    lead=cfg("OLEAD", 1))
        return _

    ou = xs.bitcast(U32)

    def out_copy(m):
        cols = pl.ds(pl.multiple_of(m * 128, 128), 128)
        return pltpu.make_async_copy(xs.at[m], out_ref.at[:, cols], sems.at[m])

    def final_block(m, _):
        rows = pl.ds(pl.multiple_of(m * 128, 128), 128)
        w = _ld(woT, (m * 128, 128), lead=(1,))
        pend = None
        for r in range(9):
            res = None
            if r < 8:
                rhs = jnp.concatenate([_ld(oT, slice(0, D), slice(r * 128, (r + 1) * 128)),
                                       _ld(oT, slice(0, D), slice(1024 + r * 128, 1152 + r * 128))],
                                      axis=1)
                res = _dot(w, rhs)
            if pend is not None:
                c0 = PAD + (r - 1) * 128
                even = xT[rows, c0:c0 + 128] + pend[:, :128]
                odd = xT[rows, 1024 + c0:1152 + c0] + pend[:, 128:]
                word = pltpu.pack_elementwise([even, odd], packed_dtype=BF16)
                ou[m, pl.ds(r - 1, 128, stride=8), :] = word.T
            pend = res
        out_copy(m).start()
        return _

    def layer_body(layer, _):
        @pl.when(layer % 2 == 0)
        def _a():
            lax.fori_loop(0, 8 // cfg('U1', 1), functools.partial(a_phase1, layer, cfg('U1', 1)), None)
            kv_tail(7)
            _drain(a_finalize_pieces(7))

            @pl.when(layer == 0)
            def _wait():
                for c in wo_cp:
                    c.wait()

            _loop(NCH, a_phase2, cfg('U2', 2))
            q_tail()

        @pl.when(layer % 2 == 1)
        def _b():
            _loop(8, b_unit, cfg('UB', 1))
            _drain(attn_pieces(1, 3, 1))

        @pl.when(layer < 3)
        def _o():
            _loop(NCH, functools.partial(o_chunk, layer), cfg('UO', 2))
            _drain(_normalize_pieces(xT, xnT, slice(S, S + PAD), 128, stat[0], stat[1]))

        return _

    lax.fori_loop(0, 4, layer_body, None)
    _loop(8, final_block, cfg('UF', 2))
    for m in range(8):
        out_copy(m).wait()


@jax.jit
def pallas_interleave_layers__linear_kernel_hedgehog__sliding_local_dilated__prompt_kernel(
    A_x: jax.Array,
    A_wqkv: jax.Array,
    A_w_phi: jax.Array,
    A_wo: jax.Array,
    B_x: jax.Array,
    B_wqkv: jax.Array,
    B_wo: jax.Array,
):
    del B_x
    hbm = pl.BlockSpec(memory_space=pl.ANY)
    out = pl.pallas_call(
        _kernel,
        out_shape=jax.ShapeDtypeStruct((S, D), BF16),
        in_specs=[hbm, hbm, pl.BlockSpec(memory_space=pltpu.VMEM), hbm, hbm, hbm],
        out_specs=hbm,
        scratch_shapes=[
            pltpu.VMEM((8, S, 128), BF16),
            pltpu.VMEM((D, 3 * D), BF16),
            pltpu.VMEM((D + 16, 3 * D), BF16),
            pltpu.VMEM((2 * D + 16, D), BF16),
            pltpu.VMEM((4, 128, 128), U32),
            pltpu.VMEM((D, PAD + S + 128), F32),
            pltpu.VMEM((D // 2, PAD + S + 128), U32),
            pltpu.VMEM((D // 2, S + 128), U32),
            pltpu.VMEM((D, D + cfg('WPAD', 0)), U32),
            pltpu.VMEM((D // 2, D + cfg('WPAD', 0)), U32),
            pltpu.VMEM((2, D // 2 + 8, D + cfg('WPAD', 0)), U32),
            pltpu.VMEM((8, 3 * D // 2 + 8, 128), U32),
            pltpu.VMEM((D, 128), F32),
            pltpu.VMEM((2 * D, 128), F32),
            pltpu.VMEM((2 * D, 128), F32),
            pltpu.VMEM((D // 2, 128), U32),
            pltpu.VMEM((256, NC), F32),
            pltpu.VMEM((16, NC), F32),
            pltpu.VMEM((2, 8, NC), F32),
            pltpu.VMEM((D // 2, 128), U32),
            pltpu.VMEM((2, 256, 1024 + cfg('QPAD', 128)), F32),
            pltpu.VMEM((2, 256, 1920), F32),
            pltpu.VMEM((2, 256, 1920), F32),
            pltpu.SemaphoreType.DMA((17,)),
        ],
        compiler_params=pltpu.CompilerParams(vmem_limit_bytes=110 * 2**20),
    )(A_x.reshape(S, D), A_wqkv, A_w_phi.reshape(H * DH, DH), A_wo, B_wqkv, B_wo)
    return out.reshape(1, S, D)
```

```python
import functools

import jax
import jax.numpy as jnp
from jax import lax
import jax.experimental.pallas as pl
import jax.experimental.pallas.tpu as pltpu

F32, BF16, U32 = jnp.float32, jnp.bfloat16, jnp.uint32
S, D, H, DH = 2048, 1024, 32, 32
NT = S // 128
NC = 256
NCH = S // NC
LOG2E = 1.4426950408889634
KOFF, VOFF, QDUM = 1024, 1024 + 1920, 1024 + 2 * 1920
PAD = NC
DUM = PAD + S
CFG = {}
def cfg(k, d): return CFG.get(k, d)
OM = cfg("OM", 128)
OPIPE = cfg("OPIPE", 0)
QM = cfg("QM", 256)
LM = cfg("LM", 64)
QPIPE = cfg("QPIPE", 0)
NT_DIMS = (((1,), (1,)), ((), ()))


def _dot(a, b):
    return jnp.dot(a, b, preferred_element_type=F32)


def _dot_nt(a, b):
    return lax.dot_general(a, b, NT_DIMS, preferred_element_type=F32)


def _ld(ref, rows, cols=slice(0, D), lead=()):
    if isinstance(rows, slice):
        a = rows.start or 0
        rows = slice(a // 2, None if rows.stop is None else rows.stop // 2)
    else:
        start, size = rows
        rows = pl.ds(pl.multiple_of(start // 2, 8), size // 2)
    return pltpu.bitcast(ref[lead + (rows, cols)], BF16)


def _st(ref, rows, cols, val, lead=()):
    if isinstance(rows, slice):
        rows = slice(rows.start // 2, rows.stop // 2)
    else:
        start, size = rows
        rows = pl.ds(pl.multiple_of(start // 2, 8), size // 2)
    ref[lead + (rows, cols)] = pltpu.bitcast(val, U32)


def _interleave(main, n_main, *sides, lead=0):
    done = [0] * len(sides)
    for i in range(n_main):
        next(main)
        for k, (g, n) in enumerate(sides):
            while done[k] < min(n, (i + 1) * n // (n_main - lead)):
                next(g)
                done[k] += 1
    for g in (main,) + tuple(g for g, _ in sides):
        for _ in g:
            raise AssertionError("generator piece count mismatch")


def _loop(n, body, unroll=1):
    def group(i, _):
        for u in range(unroll):
            body(i * unroll + u, None)
        return _
    lax.fori_loop(0, n // unroll, group, None)


def _drain(g):
    for _ in g:
        pass


def _red_h2(x, op):
    r = op(x[0], x[1])
    for i in range(2, 8):
        r = op(r, x[i])
    r = op(r, pltpu.roll(r, 4, 0))
    r = op(r, pltpu.roll(r, 2, 0))
    return r[None]


def _hedgehog(p):
    n = p.shape[1]
    p3 = p.reshape(8, 8, n)
    mx = _red_h2(p3, jnp.maximum)
    mn = _red_h2(p3, jnp.minimum)
    e1 = jnp.exp2(p3 - mx)
    e2 = jnp.exp2(mn - p3)
    s1 = _red_h2(e1, jnp.add)
    s2 = _red_h2(e2, jnp.add)
    a = (e1 * pl.reciprocal(s1, approx=True)).reshape(64, n)
    b = (e2 * pl.reciprocal(s2, approx=True)).reshape(64, n)
    return a, b


def _normalize_pieces(xT, xnT, cols, lm, s1, s2):
    mean = jnp.sum(s1, axis=0, keepdims=True) * (1.0 / D)
    var = jnp.maximum(jnp.sum(s2, axis=0, keepdims=True) * (1.0 / D) - mean * mean, 0.0)
    rstd = lax.rsqrt(var + 1e-5)
    for m in range(D // lm):
        r = slice(m * lm, (m + 1) * lm)
        _st(xnT, r, cols, ((xT[r, cols] - mean) * rstd).astype(BF16))
        yield


def _kernel(x_hbm, wa_hbm, wphi_ref, woa_hbm, wb_hbm, wob_hbm, out_ref,
            xs, wraw_a, wraw_b, wraw_o, tmp,
            xT, xnT, oT, wa_kv, wa_q, woT, wb,
            kvacc, zacc, zb, kvm, carry, carry_inv, stat, folds, qbuf, kbuf, vbuf, sems):

    x_cp = [pltpu.make_async_copy(x_hbm.at[:, i * 128:(i + 1) * 128], xs.at[i], sems.at[i])
            for i in range(8)]

    def wa_copies(gp):
        cols = [pl.ds(pl.multiple_of(part * D + gp * 128, 128), 128) for part in (1, 2, 0)]
        return [pltpu.make_async_copy(wa_hbm.at[:, c], wraw_a.at[:, c], sems.at[8 + gp]) for c in cols]

    def wb_copies(gp):
        cps = []
        for i in range(3):
            u = gp * 3 + i
            blk = (pl.ds(pl.multiple_of((u % 2) * 512, 512), 512),
                   pl.ds(pl.multiple_of((u // 2) * 256, 256), 256))
            cps.append(pltpu.make_async_copy(wb_hbm.at[blk], wraw_b.at[blk], sems.at[17 + gp]))
        return cps

    EARLY = cfg("EARLY", 3)

    wo_cp = [pltpu.make_async_copy(woa_hbm, wraw_o.at[0:D], sems.at[16]),
             pltpu.make_async_copy(wob_hbm, wraw_o.at[D:2 * D], sems.at[16])]
    for c in x_cp:
        c.start()
    def start_w():
        for gp in range(EARLY):
            for c in wa_copies(gp):
                c.start()
        for gp in range(8):
            for c in wb_copies(gp) + (wa_copies(gp) if gp >= EARLY else []):
                c.start()
        for c in wo_cp:
            c.start()

    if not cfg("WLATE", 0):
        start_w()

    xT[:, 0:PAD] = jnp.zeros((D, PAD), F32)
    carry[...] = jnp.zeros(carry.shape, F32)
    carry_inv[...] = jnp.zeros(carry_inv.shape, F32)
    stat[...] = jnp.zeros(stat.shape, F32)
    zacc[7 * 256:8 * 256, :] = jnp.zeros((256, 128), F32)
    kvacc[7 * 128:8 * 128, :] = jnp.zeros((128, 128), F32)
    def clear(i, _):
        rows = pl.ds(pl.multiple_of(i * 8, 8), 8)
        for buf in (qbuf, kbuf, vbuf):
            buf[1, rows, :] = jnp.zeros((8, buf.shape[2]), F32)
        return _
    lax.fori_loop(0, 32, clear, None)

    row = lax.broadcasted_iota(jnp.int32, (128, 128), 0)
    col = lax.broadcasted_iota(jnp.int32, (128, 128), 1)
    src_head = 2 * (row // 64) + row % 2
    src_j = (row % 64) // 2
    perm_h2 = ((src_head * 32 + src_j) == col).astype(BF16)
    sel_f = (lax.broadcasted_iota(jnp.int32, (128, 32), 0) % 64 // 2
             == lax.broadcasted_iota(jnp.int32, (128, 32), 1)).astype(BF16)

    def make_fold(blk, _):
        c0 = pl.multiple_of(blk * 128, 128)
        wphi = wphi_ref[pl.ds(c0, 128), :]
        fold = jnp.where(src_head == col // 32, _dot_nt(sel_f, wphi), 0.0).astype(BF16)
        _st(folds, (c0, 128), slice(0, 128), fold)
        return _

    lax.fori_loop(0, 8, make_fold, None)

    for c in x_cp:
        c.wait()
    if cfg("WLATE", 0):
        start_w()
    def x_prep():
        xu = xs.bitcast(U32)
        for r in range(8):
            sums = [None] * 4
            for i in range(8):
                t = xu[i, pl.ds(r, 128, stride=8), :].T
                halves = (pltpu.bitcast(t << 16, F32), pltpu.bitcast(t & jnp.uint32(0xFFFF0000), F32))
                for par, v in enumerate(halves):
                    c0 = PAD + par * 1024 + r * 128
                    xT[i * 128:(i + 1) * 128, c0:c0 + 128] = v
                    for k, u in enumerate((v, v * v)):
                        u = jnp.sum(u.reshape(16, 8, 128), axis=0)
                        sums[2 * par + k] = u if i == 0 else sums[2 * par + k] + u
            for par in range(2):
                c0 = PAD + par * 1024 + r * 128
                _drain(_normalize_pieces(xT, xnT, slice(c0, c0 + 128), 128, *sums[2 * par:2 * par + 2]))
            if r % 2 == 1 and r // 2 < EARLY:
                for c in wa_copies(r // 2):
                    c.wait()
                prep_a(r // 2)


    def prep_a(blk):
        c0 = pl.multiple_of(blk * 128, 128)
        fold = _ld(folds, (c0, 128), slice(0, 128))
        k = (_dot_nt(fold, wraw_a[:, pl.ds(D + c0, 128)]) * LOG2E).astype(BF16)
        v = _dot_nt(perm_h2, wraw_a[:, pl.ds(2 * D + c0, 128)]).astype(BF16)
        q = _dot_nt(fold, wraw_a[:, pl.ds(c0, 128)]) * LOG2E
        r0 = pl.multiple_of(blk * 256, 256)
        _st(wa_kv, (r0, 64), slice(0, D), k[:64])
        _st(wa_kv, (r0 + 64, 64), slice(0, D), v[:64])
        _st(wa_kv, (r0 + 128, 64), slice(0, D), k[64:])
        _st(wa_kv, (r0 + 192, 64), slice(0, D), v[64:])
        _st(wa_q, (c0, 128), slice(0, D), q.astype(BF16))

    x_prep()

    def prep_wb_pieces(gp):
        for i in range(3):
            u = gp * 3 + i
            kh, grp = u % 2, u // 2
            base = pl.multiple_of((grp % 4) * 384 + (grp // 4) * 128, 128)
            for half in range(2):
                w = wraw_b[pl.ds(pl.multiple_of(kh * 512, 512), 512),
                           pl.ds(pl.multiple_of(grp * 256 + half * 128, 128), 128)]
                t = w.astype(F32).T
                for j in range(2):
                    p = pltpu.pack_elementwise([t[64 * j:64 * j + 32], t[64 * j + 32:64 * j + 64]],
                                               packed_dtype=BF16)
                    for kt in range(4):
                        v = wb.at[kh * 4 + kt, pl.ds(base, 128), :]
                        v[pl.ds(half * 2 + j, 32, stride=4), :] = p[:, kt * 128:(kt + 1) * 128]
                yield

    def prep_wo_pieces(j):
        r0 = pl.multiple_of(j * 128, 128)
        for n in range(0, 8, WG):
            for i in range(n, n + WG):
                w = wraw_o[pl.ds(r0, 128), i * 128:(i + 1) * 128].astype(F32)
                p = jnp.concatenate(
                    [pltpu.pack_elementwise([w[64 * gl:64 * gl + 32], w[64 * gl + 32:64 * gl + 64]],
                                            packed_dtype=BF16) for gl in range(2)], axis=0)
                wp = pltpu.bitcast(p, BF16)
                _st(woT, slice(i * 128, (i + 1) * 128), pl.ds(r0, 128), wp.T, lead=(0,))
            yield
        hg, nh = j // 2, j % 2
        rb = pl.multiple_of(D + hg * 256, 256)
        for n in range(0, 4, WG):
            for i in range(n, n + WG):
                cols = pl.ds(pl.multiple_of(nh * 512 + i * 128, 128), 128)
                w = wraw_o[pl.ds(rb, 256), cols].astype(F32)
                for jj in range(4):
                    tmp[i, pl.ds(jj, 32, stride=4), :] = pltpu.pack_elementwise(
                        [w[64 * jj:64 * jj + 32], w[64 * jj + 32:64 * jj + 64]], packed_dtype=BF16)
            for i in range(n, n + WG):
                wp = pltpu.bitcast(tmp[i], BF16)
                _st(woT, (nh * 512 + i * 128, 128), pl.ds(pl.multiple_of(hg * 256, 256), 256),
                    wp.T, lead=(1,))
            yield

    WG = cfg('WG', 1)
    N_PWO = 12 // WG
    N_PWB = 6

    def a_finalize_pieces(gp):
        for gl in range(2):
            g = gp * 2 + gl
            r0 = pl.multiple_of(g * 128, 128)
            z = jnp.sum(zacc[pl.ds(r0, 128), :], axis=1, keepdims=True)
            zb[pl.ds(r0, 128), :] = jnp.broadcast_to(z, (128, 128))
            r1 = pl.multiple_of(g * 64, 64)
            same = (lax.broadcasted_iota(jnp.int32, (64, 128), 0) % 2
                    == lax.broadcasted_iota(jnp.int32, (64, 128), 1) % 2)
            _st(kvm, (r1, 64), slice(None), jnp.where(same, kvacc[pl.ds(r1, 64), :], 0.0).astype(BF16))
            yield

    def kv_epilogue(res):
        a, b = _hedgehog(res[:64])
        phi = jnp.concatenate([a, b], axis=0)
        zt = phi[:, :128] + phi[:, 128:]
        kt = _dot_nt(res[64:].astype(BF16), phi.astype(BF16))
        return zt, kt, a

    def kv_tail(gp):
        zt, kt, a = kv_epilogue(carry[0:128])
        g = gp * 2 + 1
        zacc[pl.ds(pl.multiple_of(g * 128, 128), 128), :] += zt
        kvacc[pl.ds(pl.multiple_of(g * 64, 64), 64), :] += kt
        return a

    def kv_pieces(gp):
        seq = [(gl, c) for gl in range(2) for c in range(NCH)]
        pend = None
        kv = z = None
        for i in range(len(seq)):
            gl, c = seq[i]
            res = _dot(_ld(wa_kv, (gp * 256 + gl * 128, 128)),
                       _ld(xnT, slice(0, D), slice(PAD + c * NC, PAD + (c + 1) * NC)))
            if pend is None:
                a = kv_tail((gp + 7) % 8)
            else:
                gl, c = seq[i - 1]
                zt, kt, a = kv_epilogue(pend)
                z = zt if c == 0 else z + zt
                kv = kt if c == 0 else kv + kt
                if c == NCH - 1 or i == len(seq) - 1:
                    g = gp * 2 + gl
                    zacc[pl.ds(pl.multiple_of(g * 128, 128), 128), :] = z
                    kvacc[pl.ds(pl.multiple_of(g * 64, 64), 64), :] = kv
            wraw_b[D:D + 16, 0:128] = a[0:16, 0:128].astype(BF16)
            wb[0, 1536:1544, :] = pltpu.bitcast(a[0:8, 0:128], U32)
            yield
            pend = res
        carry[0:128] = pend

    def a_phase1(layer, n, i, _):
        @pl.when(layer == 0)
        def _prep():
            for c in wb_copies(i):
                c.wait()

            @pl.when(i >= EARLY)
            def _():
                for c in wa_copies(i):
                    c.wait()
                prep_a(i)

        for u in range(n):
            gp = i * n + u
            _interleave(kv_pieces(gp), 2 * NCH, (prep_wb_pieces(gp), N_PWB),
                        (a_finalize_pieces((gp + 7) % 8), 2), lead=cfg("P1LEAD", 1))
        return _

    GQ = cfg("GQ", 2)
    QW = cfg("QW", 128)

    def q_features(g, pq):
        a, b = _hedgehog(pq)
        za = zb[g * 128:g * 128 + 64, :]
        zn = zb[g * 128 + 64:(g + 1) * 128, :]
        za = jnp.concatenate([za] * (QW // 128), axis=1)
        zn = jnp.concatenate([zn] * (QW // 128), axis=1)
        den = _red_h2((a * za + b * zn).reshape(8, 8, QW), jnp.add)
        inv = pl.reciprocal(den + 1e-6, approx=True)
        phi = jnp.concatenate([a, b], axis=0).astype(BF16)
        return _dot(_ld(kvm, slice(g * 64, (g + 1) * 64), slice(0, 128)), phi), inv, phi

    def q_store(g, cols, num, inv):
        o = (num.reshape(8, 8, QW) * inv).reshape(64, QW)
        _st(oT, slice(g * 64, (g + 1) * 64), cols, o.astype(BF16))

    QN_ROWS = 64 * GQ

    def q_carry_in():
        pq = carry[0:QN_ROWS, 0:QW]
        pn = [(carry[QN_ROWS + 64 * t:QN_ROWS + 64 * (t + 1), 0:QW],
               carry_inv[8 * t:8 * (t + 1), 0:QW][None]) for t in range(GQ)]
        return pq, pn

    def q_pieces(j):
        steps = [(w, g) for w in range(NC // QW) for g in range(0, 16, GQ)]

        def ocols(i):
            if i >= 0:
                return pl.ds(pl.multiple_of(j * NC + steps[i][0] * QW, QW), QW)
            return pl.ds(pl.multiple_of(((j + NCH - 1) % NCH) * NC + NC - QW, QW), QW)

        pq, pn = q_carry_in()
        for i, (w, g) in enumerate(steps):
            xcols = pl.ds(pl.multiple_of(PAD + j * NC + w * QW, QW), QW)
            res = _dot(_ld(wa_q, slice(g * 64, g * 64 + QN_ROWS)), _ld(xnT, slice(0, D), xcols))
            new = []
            for t in range(GQ):
                num, inv, phi = q_features(steps[i - 1][1] + t, pq[64 * t:64 * (t + 1)])
                q_store(steps[i - 2][1] + t, ocols(i - 2), *pn[t])
                new.append((num, inv))
            pq, pn = res, new
            anchor = phi[0:16, 0:128]
            wraw_o[2 * D:2 * D + 16, 0:128] = anchor
            woT[0, 512:520, 0:128] = pltpu.bitcast(anchor, U32)
            yield
        carry[0:QN_ROWS, 0:QW] = pq
        for t in range(GQ):
            carry[QN_ROWS + 64 * t:QN_ROWS + 64 * (t + 1), 0:QW] = pn[t][0]
            carry_inv[8 * t:8 * (t + 1), 0:QW] = pn[t][1][0]

    def q_tail():
        cols = slice(S - QW, S)
        pq, pn = q_carry_in()
        for t in range(GQ):
            num, inv, _phi = q_features(16 - GQ + t, pq[64 * t:64 * (t + 1)])
            q_store(16 - 2 * GQ + t, cols, *pn[t])
            q_store(16 - GQ + t, cols, num, inv)

    def a_phase2(j, _):
        _interleave(q_pieces(j), (16 // GQ) * (NC // QW), (prep_wo_pieces(j), N_PWO), lead=cfg("P2LEAD", 2))
        return _

    QN = cfg("QN", 128)

    def qkv_pieces(par, hg, slot):
        per = 256 // QM
        for n in range(1024 // QN):
            xcols = pl.ds(pl.multiple_of(PAD + par * 1024 + n * QN, 128), QN)
            for m in range(3 * per):
                rp0 = pl.multiple_of(hg * 384 + m * (QM // 2), QM // 2)
                w = jnp.concatenate([pltpu.bitcast(wb[kt, pl.ds(rp0, QM // 2), :], BF16)
                                     for kt in range(8)], axis=1)
                res = _dot(w, _ld(xnT, slice(0, D), xcols))
                rr = slice((m % per) * QM, (m % per) * QM + QM)
                if m < per:
                    qbuf[slot, rr, n * QN:(n + 1) * QN] = res
                else:
                    buf = kbuf if m < 2 * per else vbuf
                    buf[slot, rr, 896 + n * QN:896 + (n + 1) * QN] = res
                    for i in range(QN // 128):
                        t = n * (QN // 128) + i
                        if t >= 1:
                            buf[slot, rr, (t - 1) * 128:t * 128] = pltpu.roll(
                                res[:, i * 128:(i + 1) * 128], 1, 1)
                yield

    N_QKV = (1024 // QN) * (768 // QM)
    lane0 = lax.broadcasted_iota(jnp.int32, (8, 128), 1) == 0

    def attn_pieces(par, hg, slot):
        scale = DH ** -0.5 * LOG2E
        for rp in range(0, 8, 2):
            logit = [[None] * 8, [None] * 8]
            for dd in range(0, 32, 8):
                for d in range(dd, dd + 8):
                    rows = slice(d * 8, d * 8 + 8)
                    q = [qbuf[slot, rows, (rp + a) * 128:(rp + a + 1) * 128] for a in range(2)]
                    for e in range(rp, rp + 9):
                        k = kbuf[slot, rows, e * 128:(e + 1) * 128]
                        for a in range(2):
                            w = rp + a + 7 - e
                            if 0 <= w < 8:
                                t = q[a] * k
                                logit[a][w] = t if logit[a][w] is None else logit[a][w] + t
                yield
            prob = []
            for a in range(2):
                lg = []
                for w in range(8):
                    t = logit[a][w] * scale
                    if w > rp + a:
                        t = jnp.where(lane0, -1e9 * LOG2E, t)
                    lg.append(t)
                mx = functools.reduce(jnp.maximum, lg)
                ex = [jnp.exp2(t - mx) for t in lg]
                inv = pl.reciprocal(functools.reduce(jnp.add, ex), approx=True)
                prob.append([t * inv for t in ex])
            yield
            for dd in range(0, 32, 2):
                outs = []
                for d in (dd, dd + 1):
                    rows = slice(d * 8, d * 8 + 8)
                    acc = [None, None]
                    for e in range(rp, rp + 9):
                        v = vbuf[slot, rows, e * 128:(e + 1) * 128]
                        for a in range(2):
                            w = rp + a + 7 - e
                            if 0 <= w < 8:
                                t = prob[a][w] * v
                                acc[a] = t if acc[a] is None else acc[a] + t
                    outs.append(jnp.concatenate(acc, axis=1))
                o = jnp.concatenate(outs, axis=0).astype(BF16)
                r0 = pl.multiple_of(hg * 256 + dd * 8, 16)
                c0 = pl.multiple_of(par * 1024 + rp * 128, 256)
                _st(oT, (r0, 16), pl.ds(c0, 256), o)
                if dd % 8 == 6:
                    yield

    N_ATTN = 4 * 9

    def b_unit(i, _):
        prev = (i + 7) % 8
        _interleave(qkv_pieces(i // 4, i % 4, i % 2), N_QKV,
                    (attn_pieces(prev // 4, prev % 4, prev % 2), N_ATTN), lead=cfg("BLEAD", 1))
        return _

    ON = cfg("ON", 256)

    def oproj_pieces(layer, c0, xv):
        for n in range(NC // ON):
            s1 = s2 = None
            xc = slice(NC + n * ON, NC + (n + 1) * ON)
            for m in range(D // OM):
                rows = slice(m * OM, (m + 1) * OM)
                res = _dot(_ld(woT, rows, lead=(layer % 2,)),
                           _ld(oT, slice(0, D), pl.ds(pl.multiple_of(c0 + n * ON, 128), ON)))
                x = xv[rows, xc] + res
                xv[rows, xc] = x
                t1 = jnp.sum(x.reshape(OM // 8, 8, ON), axis=0)
                t2 = jnp.sum((x * x).reshape(OM // 8, 8, ON), axis=0)
                s1, s2 = (t1, t2) if m == 0 else (s1 + t1, s2 + t2)
                xnT[0:8, DUM:DUM + 128] = pltpu.bitcast(res[OM - 8:, ON - 128:], U32)
                xT[0:8, DUM:DUM + 128] = res[OM - 8:, ON - 128:]
                yield
            stat[0, :, n * ON:(n + 1) * ON] = s1
            stat[1, :, n * ON:(n + 1) * ON] = s2

    def o_chunk(layer, j, _):
        c0 = pl.multiple_of(j * NC, NC)
        xv = xT.at[:, pl.ds(c0, 2 * NC)]
        xnv = xnT.at[:, pl.ds(c0, 2 * NC)]
        _interleave(oproj_pieces(layer, c0, xv), (D // OM) * (NC // ON),
                    (_normalize_pieces(xv, xnv, slice(0, NC), LM, stat[0], stat[1]), D // LM),
                    lead=cfg("OLEAD", 1))
        return _

    ou = xs.bitcast(U32)

    def out_copy(m):
        cols = pl.ds(pl.multiple_of(m * 128, 128), 128)
        return pltpu.make_async_copy(xs.at[m], out_ref.at[:, cols], sems.at[m])

    def final_block(m, _):
        rows = pl.ds(pl.multiple_of(m * 128, 128), 128)
        w = _ld(woT, (m * 128, 128), lead=(1,))
        pend = None
        for r in range(9):
            res = None
            if r < 8:
                rhs = jnp.concatenate([_ld(oT, slice(0, D), slice(r * 128, (r + 1) * 128)),
                                       _ld(oT, slice(0, D), slice(1024 + r * 128, 1152 + r * 128))],
                                      axis=1)
                res = _dot(w, rhs)
            if pend is not None:
                c0 = PAD + (r - 1) * 128
                even = xT[rows, c0:c0 + 128] + pend[:, :128]
                odd = xT[rows, 1024 + c0:1152 + c0] + pend[:, 128:]
                word = pltpu.pack_elementwise([even, odd], packed_dtype=BF16)
                ou[m, pl.ds(r - 1, 128, stride=8), :] = word.T
            pend = res
        out_copy(m).start()
        return _

    def layer_body(layer, _):
        @pl.when(layer % 2 == 0)
        def _a():
            lax.fori_loop(0, 8 // cfg('U1', 1), functools.partial(a_phase1, layer, cfg('U1', 1)), None)
            kv_tail(7)
            _drain(a_finalize_pieces(7))

            @pl.when(layer == 0)
            def _wait():
                for c in wo_cp:
                    c.wait()

            _loop(NCH, a_phase2, cfg('U2', 2))
            q_tail()

        @pl.when(layer % 2 == 1)
        def _b():
            _loop(8, b_unit, cfg('UB', 1))
            _drain(attn_pieces(1, 3, 1))

        @pl.when(layer < 3)
        def _o():
            _loop(NCH, functools.partial(o_chunk, layer), cfg('UO', 2))
            _drain(_normalize_pieces(xT, xnT, slice(S, S + PAD), 128, stat[0], stat[1]))

        return _

    lax.fori_loop(0, 4, layer_body, None)
    _loop(8, final_block, cfg('UF', 2))
    for m in range(8):
        out_copy(m).wait()


@jax.jit
def pallas_interleave_layers__linear_kernel_hedgehog__sliding_local_dilated__prompt_kernel(
    A_x: jax.Array,
    A_wqkv: jax.Array,
    A_w_phi: jax.Array,
    A_wo: jax.Array,
    B_x: jax.Array,
    B_wqkv: jax.Array,
    B_wo: jax.Array,
):
    del B_x
    hbm = pl.BlockSpec(memory_space=pl.ANY)
    out = pl.pallas_call(
        _kernel,
        out_shape=jax.ShapeDtypeStruct((S, D), BF16),
        in_specs=[hbm, hbm, pl.BlockSpec(memory_space=pltpu.VMEM), hbm, hbm, hbm],
        out_specs=hbm,
        scratch_shapes=[
            pltpu.VMEM((8, S, 128), BF16),
            pltpu.VMEM((D, 3 * D), BF16),
            pltpu.VMEM((D + 16, 3 * D), BF16),
            pltpu.VMEM((2 * D + 16, D), BF16),
            pltpu.VMEM((4, 128, 128), U32),
            pltpu.VMEM((D, PAD + S + 128), F32),
            pltpu.VMEM((D // 2, PAD + S + 128), U32),
            pltpu.VMEM((D // 2, S + 128), U32),
            pltpu.VMEM((D, D + cfg('WPAD', 0)), U32),
            pltpu.VMEM((D // 2, D + cfg('WPAD', 0)), U32),
            pltpu.VMEM((2, D // 2 + 8, D + cfg('WPAD', 0)), U32),
            pltpu.VMEM((8, 3 * D // 2 + 8, 128), U32),
            pltpu.VMEM((D, 128), F32),
            pltpu.VMEM((2 * D, 128), F32),
            pltpu.VMEM((2 * D, 128), F32),
            pltpu.VMEM((D // 2, 128), U32),
            pltpu.VMEM((512, NC), F32),
            pltpu.VMEM((32, NC), F32),
            pltpu.VMEM((2, 8, NC), F32),
            pltpu.VMEM((D // 2, 128), U32),
            pltpu.VMEM((2, 256, 1024 + cfg('QPAD', 128)), F32),
            pltpu.VMEM((2, 256, 1920), F32),
            pltpu.VMEM((2, 256, 1920), F32),
            pltpu.SemaphoreType.DMA((25,)),
        ],
        compiler_params=pltpu.CompilerParams(vmem_limit_bytes=110 * 2**20),
    )(A_x.reshape(S, D), A_wqkv, A_w_phi.reshape(H * DH, DH), A_wo, B_wqkv, B_wo)
    return out.reshape(1, S, D)
```

```python
import functools

import jax
import jax.numpy as jnp
from jax import lax
import jax.experimental.pallas as pl
import jax.experimental.pallas.tpu as pltpu

F32, BF16, U32 = jnp.float32, jnp.bfloat16, jnp.uint32
S, D, H, DH = 2048, 1024, 32, 32
NT = S // 128
NC = 256
NCH = S // NC
LOG2E = 1.4426950408889634
KOFF, VOFF, QDUM = 1024, 1024 + 1920, 1024 + 2 * 1920
PAD = NC
DUM = PAD + S
CFG = {}
def cfg(k, d): return CFG.get(k, d)
OM = cfg("OM", 128)
OPIPE = cfg("OPIPE", 0)
QM = cfg("QM", 256)
LM = cfg("LM", 64)
QPIPE = cfg("QPIPE", 0)
NT_DIMS = (((1,), (1,)), ((), ()))


def _dot(a, b):
    return jnp.dot(a, b, preferred_element_type=F32)


def _dot_nt(a, b):
    return lax.dot_general(a, b, NT_DIMS, preferred_element_type=F32)


def _ld(ref, rows, cols=slice(0, D), lead=()):
    if isinstance(rows, slice):
        a = rows.start or 0
        rows = slice(a // 2, None if rows.stop is None else rows.stop // 2)
    else:
        start, size = rows
        rows = pl.ds(pl.multiple_of(start // 2, 8), size // 2)
    return pltpu.bitcast(ref[lead + (rows, cols)], BF16)


def _st(ref, rows, cols, val, lead=()):
    if isinstance(rows, slice):
        rows = slice(rows.start // 2, rows.stop // 2)
    else:
        start, size = rows
        rows = pl.ds(pl.multiple_of(start // 2, 8), size // 2)
    ref[lead + (rows, cols)] = pltpu.bitcast(val, U32)


def _interleave(main, n_main, *sides, lead=0, lag=0):
    done = [0] * len(sides)
    for i in range(n_main):
        next(main)
        for k, (g, n) in enumerate(sides):
            while done[k] < min(n, max(i + 1 - lag, 0) * n // (n_main - lead - lag)):
                next(g)
                done[k] += 1
    for g in (main,) + tuple(g for g, _ in sides):
        for _ in g:
            raise AssertionError("generator piece count mismatch")


def _loop(n, body, unroll=1):
    def group(i, _):
        for u in range(unroll):
            body(i * unroll + u, None)
        return _
    lax.fori_loop(0, n // unroll, group, None)


def _drain(g):
    for _ in g:
        pass


def _red_h2(x, op):
    r = op(x[0], x[1])
    for i in range(2, 8):
        r = op(r, x[i])
    r = op(r, pltpu.roll(r, 4, 0))
    r = op(r, pltpu.roll(r, 2, 0))
    return r[None]


def _hedgehog(p):
    n = p.shape[1]
    p3 = p.reshape(8, 8, n)
    mx = _red_h2(p3, jnp.maximum)
    mn = _red_h2(p3, jnp.minimum)
    e1 = jnp.exp2(p3 - mx)
    e2 = jnp.exp2(mn - p3)
    s1 = _red_h2(e1, jnp.add)
    s2 = _red_h2(e2, jnp.add)
    a = (e1 * pl.reciprocal(s1, approx=True)).reshape(64, n)
    b = (e2 * pl.reciprocal(s2, approx=True)).reshape(64, n)
    return a, b


def _normalize_pieces(xT, xnT, cols, lm, s1, s2):
    mean = jnp.sum(s1, axis=0, keepdims=True) * (1.0 / D)
    var = jnp.maximum(jnp.sum(s2, axis=0, keepdims=True) * (1.0 / D) - mean * mean, 0.0)
    rstd = lax.rsqrt(var + 1e-5)
    for m in range(D // lm):
        r = slice(m * lm, (m + 1) * lm)
        _st(xnT, r, cols, ((xT[r, cols] - mean) * rstd).astype(BF16))
        yield


def _kernel(x_hbm, wa_hbm, wphi_ref, woa_hbm, wb_hbm, wob_hbm, out_ref,
            xs, wraw_a, wraw_b, wraw_o, tmp,
            xT, xnT, oT, wa_kv, wa_q, woT, wb,
            kvacc, zacc, zb, kvm, carry, carry_inv, stat, folds, qbuf, kbuf, vbuf, sems):

    x_cp = [pltpu.make_async_copy(x_hbm.at[:, i * 128:(i + 1) * 128], xs.at[i], sems.at[i])
            for i in range(8)]

    def wa_copies(gp):
        cols = [pl.ds(pl.multiple_of(part * D + gp * 128, 128), 128) for part in (1, 2, 0)]
        return [pltpu.make_async_copy(wa_hbm.at[:, c], wraw_a.at[:, c], sems.at[8 + gp]) for c in cols]

    def wb_copies(gp):
        cps = []
        for i in range(3):
            u = gp * 3 + i
            blk = (pl.ds(pl.multiple_of((u % 2) * 512, 512), 512),
                   pl.ds(pl.multiple_of((u // 2) * 256, 256), 256))
            cps.append(pltpu.make_async_copy(wb_hbm.at[blk], wraw_b.at[blk], sems.at[17 + gp]))
        return cps

    EARLY = cfg("EARLY", 1)

    wo_cp = [pltpu.make_async_copy(woa_hbm, wraw_o.at[0:D], sems.at[16]),
             pltpu.make_async_copy(wob_hbm, wraw_o.at[D:2 * D], sems.at[16])]
    for c in x_cp:
        c.start()
    def start_w():
        for gp in range(EARLY):
            for c in wa_copies(gp):
                c.start()
        for gp in range(8):
            for c in wb_copies(gp) + (wa_copies(gp) if gp >= EARLY else []):
                c.start()
        for c in wo_cp:
            c.start()

    if not cfg("WLATE", 0):
        start_w()

    xT[:, 0:PAD] = jnp.zeros((D, PAD), F32)
    carry[...] = jnp.zeros(carry.shape, F32)
    carry_inv[...] = jnp.zeros(carry_inv.shape, F32)
    stat[...] = jnp.zeros(stat.shape, F32)
    zacc[7 * 256:8 * 256, :] = jnp.zeros((256, 128), F32)
    kvacc[7 * 128:8 * 128, :] = jnp.zeros((128, 128), F32)
    def clear(i, _):
        rows = pl.ds(pl.multiple_of(i * 8, 8), 8)
        for buf in (qbuf, kbuf, vbuf):
            buf[1, rows, :] = jnp.zeros((8, buf.shape[2]), F32)
        return _
    lax.fori_loop(0, 32, clear, None)

    row = lax.broadcasted_iota(jnp.int32, (128, 128), 0)
    col = lax.broadcasted_iota(jnp.int32, (128, 128), 1)
    src_head = 2 * (row // 64) + row % 2
    src_j = (row % 64) // 2
    perm_h2 = ((src_head * 32 + src_j) == col).astype(BF16)
    sel_f = (lax.broadcasted_iota(jnp.int32, (128, 32), 0) % 64 // 2
             == lax.broadcasted_iota(jnp.int32, (128, 32), 1)).astype(BF16)

    def make_fold(blk, _):
        c0 = pl.multiple_of(blk * 128, 128)
        wphi = wphi_ref[pl.ds(c0, 128), :]
        fold = jnp.where(src_head == col // 32, _dot_nt(sel_f, wphi), 0.0).astype(BF16)
        _st(folds, (c0, 128), slice(0, 128), fold)
        return _

    lax.fori_loop(0, 8, make_fold, None)

    if cfg("WLATE", 0):
        start_w()
    def x_prep():
        xu = xs.bitcast(U32)
        sums = [[None] * 4 for _ in range(8)]
        for i in range(8):
            x_cp[i].wait()
            for r in range(8):
                t = xu[i, pl.ds(r, 128, stride=8), :].T
                halves = (pltpu.bitcast(t << 16, F32), pltpu.bitcast(t & jnp.uint32(0xFFFF0000), F32))
                for par, v in enumerate(halves):
                    c0 = PAD + par * 1024 + r * 128
                    xT[i * 128:(i + 1) * 128, c0:c0 + 128] = v
                    for k, u in enumerate((v, v * v)):
                        u = jnp.sum(u.reshape(16, 8, 128), axis=0)
                        sums[r][2 * par + k] = u if i == 0 else sums[r][2 * par + k] + u
        for r in range(8):
            for par in range(2):
                c0 = PAD + par * 1024 + r * 128
                _drain(_normalize_pieces(xT, xnT, slice(c0, c0 + 128), 128, *sums[r][2 * par:2 * par + 2]))
            if r >= 8 - EARLY:
                for c in wa_copies(r - 8 + EARLY):
                    c.wait()
                prep_a(r - 8 + EARLY)


    def prep_a(blk):
        c0 = pl.multiple_of(blk * 128, 128)
        fold = _ld(folds, (c0, 128), slice(0, 128))
        k = (_dot_nt(fold, wraw_a[:, pl.ds(D + c0, 128)]) * LOG2E).astype(BF16)
        v = _dot_nt(perm_h2, wraw_a[:, pl.ds(2 * D + c0, 128)]).astype(BF16)
        q = _dot_nt(fold, wraw_a[:, pl.ds(c0, 128)]) * LOG2E
        r0 = pl.multiple_of(blk * 256, 256)
        _st(wa_kv, (r0, 64), slice(0, D), k[:64])
        _st(wa_kv, (r0 + 64, 64), slice(0, D), v[:64])
        _st(wa_kv, (r0 + 128, 64), slice(0, D), k[64:])
        _st(wa_kv, (r0 + 192, 64), slice(0, D), v[64:])
        _st(wa_q, (c0, 128), slice(0, D), q.astype(BF16))

    x_prep()

    def prep_wb_pieces(gp):
        for i in range(3):
            u = gp * 3 + i
            kh, grp = u % 2, u // 2
            base = pl.multiple_of((grp % 4) * 384 + (grp // 4) * 128, 128)
            for half in range(2):
                w = wraw_b[pl.ds(pl.multiple_of(kh * 512, 512), 512),
                           pl.ds(pl.multiple_of(grp * 256 + half * 128, 128), 128)]
                t = w.astype(F32).T
                for j in range(2):
                    p = pltpu.pack_elementwise([t[64 * j:64 * j + 32], t[64 * j + 32:64 * j + 64]],
                                               packed_dtype=BF16)
                    for kt in range(4):
                        v = wb.at[kh * 4 + kt, pl.ds(base, 128), :]
                        v[pl.ds(half * 2 + j, 32, stride=4), :] = p[:, kt * 128:(kt + 1) * 128]
                yield

    def prep_wo_pieces(j):
        r0 = pl.multiple_of(j * 128, 128)
        for n in range(0, 8, WG):
            for i in range(n, n + WG):
                w = wraw_o[pl.ds(r0, 128), i * 128:(i + 1) * 128].astype(F32)
                p = jnp.concatenate(
                    [pltpu.pack_elementwise([w[64 * gl:64 * gl + 32], w[64 * gl + 32:64 * gl + 64]],
                                            packed_dtype=BF16) for gl in range(2)], axis=0)
                wp = pltpu.bitcast(p, BF16)
                _st(woT, slice(i * 128, (i + 1) * 128), pl.ds(r0, 128), wp.T, lead=(0,))
            yield
        hg, nh = j // 2, j % 2
        rb = pl.multiple_of(D + hg * 256, 256)
        for n in range(0, 4, WG):
            for i in range(n, n + WG):
                cols = pl.ds(pl.multiple_of(nh * 512 + i * 128, 128), 128)
                w = wraw_o[pl.ds(rb, 256), cols].astype(F32)
                for jj in range(4):
                    tmp[i, pl.ds(jj, 32, stride=4), :] = pltpu.pack_elementwise(
                        [w[64 * jj:64 * jj + 32], w[64 * jj + 32:64 * jj + 64]], packed_dtype=BF16)
            for i in range(n, n + WG):
                wp = pltpu.bitcast(tmp[i], BF16)
                _st(woT, (nh * 512 + i * 128, 128), pl.ds(pl.multiple_of(hg * 256, 256), 256),
                    wp.T, lead=(1,))
            yield

    WG = cfg('WG', 1)
    N_PWO = 12 // WG
    N_PWB = 6

    def a_finalize_pieces(gp):
        for gl in range(2):
            g = gp * 2 + gl
            r0 = pl.multiple_of(g * 128, 128)
            z = jnp.sum(zacc[pl.ds(r0, 128), :], axis=1, keepdims=True)
            zb[pl.ds(r0, 128), :] = jnp.broadcast_to(z, (128, 128))
            r1 = pl.multiple_of(g * 64, 64)
            same = (lax.broadcasted_iota(jnp.int32, (64, 128), 0) % 2
                    == lax.broadcasted_iota(jnp.int32, (64, 128), 1) % 2)
            _st(kvm, (r1, 64), slice(None), jnp.where(same, kvacc[pl.ds(r1, 64), :], 0.0).astype(BF16))
            yield

    def kv_epilogue(res):
        a, b = _hedgehog(res[:64])
        phi = jnp.concatenate([a, b], axis=0)
        zt = phi[:, :128] + phi[:, 128:]
        kt = _dot_nt(res[64:].astype(BF16), phi.astype(BF16))
        return zt, kt, a

    def kv_tail(gp):
        zt, kt, a = kv_epilogue(carry[0:128])
        g = gp * 2 + 1
        zacc[pl.ds(pl.multiple_of(g * 128, 128), 128), :] += zt
        kvacc[pl.ds(pl.multiple_of(g * 64, 64), 64), :] += kt
        return a

    def kv_pieces(gp):
        seq = [(gl, c) for gl in range(2) for c in range(NCH)]
        pend = None
        kv = z = None
        for i in range(len(seq)):
            gl, c = seq[i]
            res = _dot(_ld(wa_kv, (gp * 256 + gl * 128, 128)),
                       _ld(xnT, slice(0, D), slice(PAD + c * NC, PAD + (c + 1) * NC)))
            if pend is None:
                a = kv_tail((gp + 7) % 8)
            else:
                gl, c = seq[i - 1]
                zt, kt, a = kv_epilogue(pend)
                z = zt if c == 0 else z + zt
                kv = kt if c == 0 else kv + kt
                if c == NCH - 1 or i == len(seq) - 1:
                    g = gp * 2 + gl
                    zacc[pl.ds(pl.multiple_of(g * 128, 128), 128), :] = z
                    kvacc[pl.ds(pl.multiple_of(g * 64, 64), 64), :] = kv
            wraw_b[D:D + 16, 0:128] = a[0:16, 0:128].astype(BF16)
            wb[0, 1536:1544, :] = pltpu.bitcast(a[0:8, 0:128], U32)
            yield
            pend = res
        carry[0:128] = pend

    def a_phase1(layer, n, i, _):
        @pl.when(layer == 0)
        def _prep():
            for c in wb_copies(i):
                c.wait()

            @pl.when(i >= EARLY)
            def _():
                for c in wa_copies(i):
                    c.wait()
                prep_a(i)

        for u in range(n):
            gp = i * n + u
            _interleave(kv_pieces(gp), 2 * NCH, (prep_wb_pieces(gp), N_PWB),
                        (a_finalize_pieces((gp + 7) % 8), 2), lead=cfg("P1LEAD", 1))
        return _

    GQ = cfg("GQ", 2)
    QW = cfg("QW", 128)

    def q_features(g, pq):
        a, b = _hedgehog(pq)
        za = zb[g * 128:g * 128 + 64, :]
        zn = zb[g * 128 + 64:(g + 1) * 128, :]
        za = jnp.concatenate([za] * (QW // 128), axis=1)
        zn = jnp.concatenate([zn] * (QW // 128), axis=1)
        den = _red_h2((a * za + b * zn).reshape(8, 8, QW), jnp.add)
        inv = pl.reciprocal(den + 1e-6, approx=True)
        phi = jnp.concatenate([a, b], axis=0).astype(BF16)
        return _dot(_ld(kvm, slice(g * 64, (g + 1) * 64), slice(0, 128)), phi), inv, phi

    def q_store(g, cols, num, inv):
        o = (num.reshape(8, 8, QW) * inv).reshape(64, QW)
        _st(oT, slice(g * 64, (g + 1) * 64), cols, o.astype(BF16))

    QN_ROWS = 64 * GQ

    def q_carry_in():
        pq = carry[0:QN_ROWS, 0:QW]
        pn = [(carry[QN_ROWS + 64 * t:QN_ROWS + 64 * (t + 1), 0:QW],
               carry_inv[8 * t:8 * (t + 1), 0:QW][None]) for t in range(GQ)]
        return pq, pn

    def q_pieces(j):
        steps = [(w, g) for w in range(NC // QW) for g in range(0, 16, GQ)]

        def ocols(i):
            if i >= 0:
                return pl.ds(pl.multiple_of(j * NC + steps[i][0] * QW, QW), QW)
            return pl.ds(pl.multiple_of(((j + NCH - 1) % NCH) * NC + NC - QW, QW), QW)

        pq, pn = q_carry_in()
        for i, (w, g) in enumerate(steps):
            xcols = pl.ds(pl.multiple_of(PAD + j * NC + w * QW, QW), QW)
            res = _dot(_ld(wa_q, slice(g * 64, g * 64 + QN_ROWS)), _ld(xnT, slice(0, D), xcols))
            new = []
            for t in range(GQ):
                num, inv, phi = q_features(steps[i - 1][1] + t, pq[64 * t:64 * (t + 1)])
                q_store(steps[i - 2][1] + t, ocols(i - 2), *pn[t])
                new.append((num, inv))
            pq, pn = res, new
            anchor = phi[0:16, 0:128]
            wraw_o[2 * D:2 * D + 16, 0:128] = anchor
            woT[0, 512:520, 0:128] = pltpu.bitcast(anchor, U32)
            yield
        carry[0:QN_ROWS, 0:QW] = pq
        for t in range(GQ):
            carry[QN_ROWS + 64 * t:QN_ROWS + 64 * (t + 1), 0:QW] = pn[t][0]
            carry_inv[8 * t:8 * (t + 1), 0:QW] = pn[t][1][0]

    def q_tail():
        cols = slice(S - QW, S)
        pq, pn = q_carry_in()
        for t in range(GQ):
            num, inv, _phi = q_features(16 - GQ + t, pq[64 * t:64 * (t + 1)])
            q_store(16 - 2 * GQ + t, cols, *pn[t])
            q_store(16 - GQ + t, cols, num, inv)

    def a_phase2(j, _):
        _interleave(q_pieces(j), (16 // GQ) * (NC // QW), (prep_wo_pieces(j), N_PWO), lead=cfg("P2LEAD", 2))
        return _

    QN = cfg("QN", 128)

    def qkv_pieces(par, hg, slot):
        per = 256 // QM
        for n in range(1024 // QN):
            xcols = pl.ds(pl.multiple_of(PAD + par * 1024 + n * QN, 128), QN)
            for m in [(t + cfg('MROT', 0)) % (3 * per) for t in range(3 * per)]:
                rp0 = pl.multiple_of(hg * 384 + m * (QM // 2), QM // 2)
                w = jnp.concatenate([pltpu.bitcast(wb[kt, pl.ds(rp0, QM // 2), :], BF16)
                                     for kt in range(8)], axis=1)
                res = _dot(w, _ld(xnT, slice(0, D), xcols))
                rr = slice((m % per) * QM, (m % per) * QM + QM)
                if m < per:
                    qbuf[slot, rr, n * QN:(n + 1) * QN] = res
                else:
                    buf = kbuf if m < 2 * per else vbuf
                    buf[slot, rr, 896 + n * QN:896 + (n + 1) * QN] = res
                    for i in range(QN // 128):
                        t = n * (QN // 128) + i
                        if t >= 1:
                            buf[slot, rr, (t - 1) * 128:t * 128] = pltpu.roll(
                                res[:, i * 128:(i + 1) * 128], 1, 1)
                yield

    N_QKV = (1024 // QN) * (768 // QM)
    lane0 = lax.broadcasted_iota(jnp.int32, (8, 128), 1) == 0

    def attn_pieces(par, hg, slot):
        scale = DH ** -0.5 * LOG2E
        for rp in range(0, 8, 2):
            logit = [[None] * 8, [None] * 8]
            for dd in range(0, 32, 8):
                for d in range(dd, dd + 8):
                    rows = slice(d * 8, d * 8 + 8)
                    q = [qbuf[slot, rows, (rp + a) * 128:(rp + a + 1) * 128] for a in range(2)]
                    for e in range(rp, rp + 9):
                        k = kbuf[slot, rows, e * 128:(e + 1) * 128]
                        for a in range(2):
                            w = rp + a + 7 - e
                            if 0 <= w < 8:
                                t = q[a] * k
                                logit[a][w] = t if logit[a][w] is None else logit[a][w] + t
                yield
            prob = []
            for a in range(2):
                lg = []
                for w in range(8):
                    t = logit[a][w] * scale
                    if w > rp + a:
                        t = jnp.where(lane0, -1e9 * LOG2E, t)
                    lg.append(t)
                mx = functools.reduce(jnp.maximum, lg)
                ex = [jnp.exp2(t - mx) for t in lg]
                inv = pl.reciprocal(functools.reduce(jnp.add, ex), approx=True)
                prob.append([t * inv for t in ex])
            yield
            for dd in range(0, 32, 2):
                outs = []
                for d in (dd, dd + 1):
                    rows = slice(d * 8, d * 8 + 8)
                    acc = [None, None]
                    for e in range(rp, rp + 9):
                        v = vbuf[slot, rows, e * 128:(e + 1) * 128]
                        for a in range(2):
                            w = rp + a + 7 - e
                            if 0 <= w < 8:
                                t = prob[a][w] * v
                                acc[a] = t if acc[a] is None else acc[a] + t
                    outs.append(jnp.concatenate(acc, axis=1))
                o = jnp.concatenate(outs, axis=0).astype(BF16)
                r0 = pl.multiple_of(hg * 256 + dd * 8, 16)
                c0 = pl.multiple_of(par * 1024 + rp * 128, 256)
                _st(oT, (r0, 16), pl.ds(c0, 256), o)
                if dd % 8 == 6:
                    yield

    N_ATTN = 4 * 9

    def b_unit(i, _):
        prev = (i + 7) % 8
        _interleave(qkv_pieces(i // 4, i % 4, i % 2), N_QKV,
                    (attn_pieces(prev // 4, prev % 4, prev % 2), N_ATTN), lead=cfg("BLEAD", 1), lag=cfg("BLAG", 0))
        return _

    ON = cfg("ON", 256)

    def oproj_pieces(layer, c0, xv):
        for n in range(NC // ON):
            s1 = s2 = None
            xc = slice(NC + n * ON, NC + (n + 1) * ON)
            for m in range(D // OM):
                rows = slice(m * OM, (m + 1) * OM)
                res = _dot(_ld(woT, rows, lead=(layer % 2,)),
                           _ld(oT, slice(0, D), pl.ds(pl.multiple_of(c0 + n * ON, 128), ON)))
                x = xv[rows, xc] + res
                xv[rows, xc] = x
                t1 = jnp.sum(x.reshape(OM // 8, 8, ON), axis=0)
                t2 = jnp.sum((x * x).reshape(OM // 8, 8, ON), axis=0)
                s1, s2 = (t1, t2) if m == 0 else (s1 + t1, s2 + t2)
                xnT[0:8, DUM:DUM + 128] = pltpu.bitcast(res[OM - 8:, ON - 128:], U32)
                xT[0:8, DUM:DUM + 128] = res[OM - 8:, ON - 128:]
                yield
            stat[0, :, n * ON:(n + 1) * ON] = s1
            stat[1, :, n * ON:(n + 1) * ON] = s2

    def o_chunk(layer, j, _):
        c0 = pl.multiple_of(j * NC, NC)
        xv = xT.at[:, pl.ds(c0, 2 * NC)]
        xnv = xnT.at[:, pl.ds(c0, 2 * NC)]
        _interleave(oproj_pieces(layer, c0, xv), (D // OM) * (NC // ON),
                    (_normalize_pieces(xv, xnv, slice(0, NC), LM, stat[0], stat[1]), D // LM),
                    lead=cfg("OLEAD", 1))
        return _

    ou = xs.bitcast(U32)

    def out_copy(m):
        cols = pl.ds(pl.multiple_of(m * 128, 128), 128)
        return pltpu.make_async_copy(xs.at[m], out_ref.at[:, cols], sems.at[m])

    def final_block(m, _):
        rows = pl.ds(pl.multiple_of(m * 128, 128), 128)
        w = _ld(woT, (m * 128, 128), lead=(1,))
        pend = None
        for r in range(9):
            res = None
            if r < 8:
                rhs = jnp.concatenate([_ld(oT, slice(0, D), slice(r * 128, (r + 1) * 128)),
                                       _ld(oT, slice(0, D), slice(1024 + r * 128, 1152 + r * 128))],
                                      axis=1)
                res = _dot(w, rhs)
            if pend is not None:
                c0 = PAD + (r - 1) * 128
                even = xT[rows, c0:c0 + 128] + pend[:, :128]
                odd = xT[rows, 1024 + c0:1152 + c0] + pend[:, 128:]
                word = pltpu.pack_elementwise([even, odd], packed_dtype=BF16)
                ou[m, pl.ds(r - 1, 128, stride=8), :] = word.T
            pend = res
        out_copy(m).start()
        return _

    def layer_body(layer, _):
        @pl.when(layer % 2 == 0)
        def _a():
            lax.fori_loop(0, 8 // cfg('U1', 1), functools.partial(a_phase1, layer, cfg('U1', 1)), None)
            kv_tail(7)
            _drain(a_finalize_pieces(7))

            @pl.when(layer == 0)
            def _wait():
                for c in wo_cp:
                    c.wait()

            _loop(NCH, a_phase2, cfg('U2', 2))
            q_tail()

        @pl.when(layer % 2 == 1)
        def _b():
            _loop(8, b_unit, cfg('UB', 1))
            _drain(attn_pieces(1, 3, 1))

        @pl.when(layer < 3)
        def _o():
            _loop(NCH, functools.partial(o_chunk, layer), cfg('UO', 2))
            _drain(_normalize_pieces(xT, xnT, slice(S, S + PAD), 128, stat[0], stat[1]))

        return _

    lax.fori_loop(0, 4, layer_body, None)
    _loop(8, final_block, cfg('UF', 2))
    for m in range(8):
        out_copy(m).wait()


@jax.jit
def pallas_interleave_layers__linear_kernel_hedgehog__sliding_local_dilated__prompt_kernel(
    A_x: jax.Array,
    A_wqkv: jax.Array,
    A_w_phi: jax.Array,
    A_wo: jax.Array,
    B_x: jax.Array,
    B_wqkv: jax.Array,
    B_wo: jax.Array,
):
    del B_x
    hbm = pl.BlockSpec(memory_space=pl.ANY)
    out = pl.pallas_call(
        _kernel,
        out_shape=jax.ShapeDtypeStruct((S, D), BF16),
        in_specs=[hbm, hbm, pl.BlockSpec(memory_space=pltpu.VMEM), hbm, hbm, hbm],
        out_specs=hbm,
        scratch_shapes=[
            pltpu.VMEM((8, S, 128), BF16),
            pltpu.VMEM((D, 3 * D), BF16),
            pltpu.VMEM((D + 16, 3 * D), BF16),
            pltpu.VMEM((2 * D + 16, D), BF16),
            pltpu.VMEM((4, 128, 128), U32),
            pltpu.VMEM((D, PAD + S + cfg('XP', 128)), F32),
            pltpu.VMEM((D // 2, PAD + S + cfg('XNP', 128)), U32),
            pltpu.VMEM((D // 2, S + cfg('OP', 0)), U32),
            pltpu.VMEM((D, D + cfg('WPAD', 0)), U32),
            pltpu.VMEM((D // 2, D + cfg('WQPAD', 0)), U32),
            pltpu.VMEM((2, D // 2 + 8, D + cfg('WOPAD', 0)), U32),
            pltpu.VMEM((8, 3 * D // 2 + 8, 128), U32),
            pltpu.VMEM((D, 128), F32),
            pltpu.VMEM((2 * D, 128), F32),
            pltpu.VMEM((2 * D, 128), F32),
            pltpu.VMEM((D // 2, 128), U32),
            pltpu.VMEM((512, NC), F32),
            pltpu.VMEM((32, NC), F32),
            pltpu.VMEM((2, 8, NC), F32),
            pltpu.VMEM((D // 2, 128), U32),
            pltpu.VMEM((2, 256, 1024 + cfg('QPAD', 128)), F32),
            pltpu.VMEM((2, 256, 1920 + cfg('KP', 0)), F32),
            pltpu.VMEM((2, 256, 1920 + cfg('VP', 0)), F32),
            pltpu.SemaphoreType.DMA((25,)),
        ],
        compiler_params=pltpu.CompilerParams(vmem_limit_bytes=110 * 2**20),
    )(A_x.reshape(S, D), A_wqkv, A_w_phi.reshape(H * DH, DH), A_wo, B_wqkv, B_wo)
    return out.reshape(1, S, D)
```
